```python
import os as _os
_os.environ.setdefault('JAX_PLATFORMS', 'cpu')
import jax
import jax.numpy as jnp

def _softmax(x, axis=-1):
    return jax.nn.softmax(x, axis=axis)

def _gelu(x):
    return jax.nn.gelu(x, approximate=True)

def _silu(x):
    return jax.nn.silu(x)

def _sigmoid(x):
    return jax.nn.sigmoid(x)

def _layernorm(x, axis=-1, eps=1e-05):
    m = jnp.mean(x, axis=axis, keepdims=True)
    v = jnp.var(x, axis=axis, keepdims=True)
    return (x - m) / jnp.sqrt(v + eps)

def _scatter_add(tgt, idx, src, axis=0):
    return tgt.at[idx].add(src)

def _segment_sum(src, seg, n):
    return jax.ops.segment_sum(src, seg, n)

class _Rng:

    def __init__(self, key):
        self._k = key

    def _next(self):
        self._k, sub = jax.random.split(self._k)
        return sub

    def normal(self, shape):
        return jax.random.normal(self._next(), shape, dtype=jnp.bfloat16)

    def randint(self, lo, hi, shape):
        return jax.random.randint(self._next(), shape, lo, hi, dtype=jnp.int32)

    def uniform(self, shape, lo=0.0, hi=1.0):
        return jax.random.uniform(self._next(), shape, jnp.bfloat16, lo, hi)

    def permutation(self, n):
        return jax.random.permutation(self._next(), n)
kernel_name = 'adaLN_cond__sliding_local_dilated__dense_activation_gelu__prompt'

def setup_inputs():
    _rng = _Rng(jax.random.key(int.from_bytes(__import__("os").urandom(4), "little")))
    _w = lambda a: (lambda t: t.astype(jnp.bfloat16) if jnp.issubdtype(t.dtype, jnp.floating) else t)(jnp.asarray(a))

    def _A_setup():
        B, S, D = (1, 2048, 576)
        return {'x': _w((lambda *s: _rng.normal(s) * 0.05)(B, S, D)), 'wqkv': _w((lambda *s: _rng.normal(s) * 0.05)(D, 3 * D)), 'wo': _w((lambda *s: _rng.normal(s) * 0.05)(D, D))}
    _A_in = _A_setup()

    def _B_setup():
        B, S, D, F = (1, 2048, 576, 4608)
        return {'x': _w((lambda *s: _rng.normal(s) * 0.05)(B, S, D)), 'w1': _w((lambda *s: _rng.normal(s) * 0.8)(D, F) * D ** (-0.5)), 'b1': _w((lambda *s: _rng.normal(s) * 0.8)(F) * 0.01), 'w2': _w((lambda *s: _rng.normal(s) * 0.8)(F, D) * F ** (-0.5)), 'b2': _w((lambda *s: _rng.normal(s) * 0.8)(D) * 0.01)}
    _B_in = _B_setup()
    return {'A_x': _A_in['x'], 'A_wqkv': _A_in['wqkv'], 'A_wo': _A_in['wo'], 'B_x': _B_in['x'], 'B_w1': _B_in['w1'], 'B_b1': _B_in['b1'], 'B_w2': _B_in['w2'], 'B_b2': _B_in['b2'], 'c': _w((lambda *s: _rng.normal(s) * 0.05)(1, 576) * 8.0), 'w_mod': _w((lambda *s: _rng.normal(s) * 0.05)(576, 6 * 576) * 576 ** (-0.5) * 8.0)}

def reference(A_x, A_wqkv, A_wo, B_x, B_w1, B_b1, B_w2, B_b2, c, w_mod):

    def _A_ref(x, wqkv, wo):
        B, S, D = x.shape
        H = 32
        Dh = D // H
        W, dil = (8, 2)
        qkv = (lambda x, *d: x.transpose(*d))((x @ wqkv).reshape(B, S, 3, H, Dh), 2, 0, 3, 1, 4)
        q, k, v = (qkv[0], qkv[1], qkv[2])
        scale = Dh ** (-0.5)
        pos = jnp.arange(S)
        off = jnp.arange(W) * dil
        idx = pos[:, None] - off[None, :]
        mask = idx >= 0
        idx_c = jnp.where(mask, idx, 0).reshape(-1)
        kg = k[:, :, idx_c, :].reshape(B, H, S, W, Dh)
        vg = v[:, :, idx_c, :].reshape(B, H, S, W, Dh)
        logits = jnp.einsum('bhsd,bhswd->bhsw', q, kg) * scale
        logits = jnp.where(mask[None, None, :, :], logits, -1000000000.0)
        attn = _softmax(logits, axis=-1)
        o = jnp.einsum('bhsw,bhswd->bhsd', attn, vg)
        return (lambda x, *d: x.transpose(*d))(o, 0, 2, 1, 3).reshape(B, S, D) @ wo

    def _B_ref(x, w1, b1, w2, b2):
        h = jnp.einsum('bsd,df->bsf', x, w1) + b1
        h = _gelu(h)
        return jnp.einsum('bsf,fd->bsd', h, w2) + b2
    x = A_x
    mod = (_silu(c) @ w_mod).reshape(c.shape[0], 6, 1, -1)
    sa, ca, ga, sb, cb, gb = (mod[:, 0].copy(), mod[:, 1].copy(), mod[:, 2].copy(), mod[:, 3].copy(), mod[:, 4].copy(), mod[:, 5].copy())
    h = _layernorm(x, axis=-1) * (1 + ca) + sa
    x = x + ga * _A_ref(h, A_wqkv, A_wo)
    h = _layernorm(x, axis=-1) * (1 + cb) + sb
    x = x + gb * _B_ref(h, B_w1, B_b1, B_w2, B_b2)
    return x
```

```python
import jax
import jax.numpy as jnp
import numpy as np
from jax import lax
from jax.experimental import pallas as pl
from jax.experimental.pallas import tpu as pltpu

f32, bf16, u32 = jnp.float32, jnp.bfloat16, jnp.uint32
add, sub, mul = lax.add, lax.sub, lax.mul

S, D, F = 2048, 576, 4608
DH, WIN = 18, 8
T = 128
NQ = 4
DB = D // 4
FC = 4 * T
NC = F // FC
NP = 49
SHARED = -1
LAST = (0, 128, 256, 416, 576)
EPS = 1e-5
LOG2E = float(np.log2(np.e))
SCALE = float(DH ** -0.5)
GS = float(np.cbrt(np.sqrt(2.0 / np.pi) * 0.044715))
GK = np.float32(np.sqrt(2.0 / np.pi) / GS)

A_TERMS = (((1, 0, 0), (1, 1, 1)), ((1, 0, 1), (-1, 1, 1)), ((1, 0, 0), (1, 0, 1)), ((1, 1, 0), (-1, 0, 0)),
           ((1, 1, 0), (1, 1, 1)), ((1, 1, 1),), ((1, 0, 0),))
B_TERMS = (((1, 0, 0), (-1, 1, 1)), ((1, 1, 0), (-1, 1, 1)), ((1, 1, 1),), ((1, 0, 1), (-1, 0, 0)),
           ((1, 0, 0),), ((1, 1, 0), (-1, 0, 0)), ((1, 0, 1), (-1, 1, 1)))
ROW_PRODUCTS = tuple(7 * a + b for a in (2, 4) for b in (2, 4))
A_SLABS = (None, (0, 0), (2, 2), (0, 1), (1, 3), (1, 0), (2, 1),
           ((0, 0), (2, 2)), ((0, 1), (1, 3)), ((1, 0), (2, 1)))
B_SLABS = (None, (0, 0), (2, 0), (0, 1), (1, 1), (1, 2), (2, 3),
           ((0, 1), (2, 3)), ((0, 0), (1, 2)), ((1, 1), (2, 0)))
SLAB_ROW = (320, 448, 512)
DEPTH_TILES = ((0, 64), (128, 192), (256, 320), (384, 448), (320, 512), (448, 512))

STORE_COST = 3
GELU_COST = 7
RUN = 7
EXPAND_COST = 2 * 55 + STORE_COST * NP


def _cast(v, dtype):
    return lax.convert_element_type(v, dtype)


def _cat(vals, axis=0):
    return lax.concatenate(list(vals), axis)


def _dot(a, b):
    return lax.dot_general(a, b, (((1,), (0,)), ((), ())), preferred_element_type=f32)


def _ld(ref, *idx):
    return pltpu.bitcast(ref.bitcast(u32)[idx], bf16)


def _rows(t, n=16, at=0):
    return slice(at + t * n, at + (t + 1) * n)


def _once(fn):
    kept = {}

    def get(*key):
        if key not in kept:
            kept[key] = fn(*key)
        return kept[key]
    return get


def _combine(term, blk):
    v = blk(*term[0][1:])
    for sign, r, c in term[1:]:
        v = (add if sign > 0 else sub)(v, blk(r, c))
    return v


def _expand(terms, blk, emit):
    for p, outer in enumerate(terms):
        part = {}
        for r in range(2):
            for c in range(2):
                part[r, c] = _combine(outer, lambda i, j: blk[2 * i + r, 2 * j + c])
                yield 2 * (len(outer) - 1)
        for n, inner in enumerate(terms):
            emit(7 * p + n, _cast(_combine(inner, lambda r, c: part[r, c]), bf16))
            yield 2 * (len(inner) - 1) + STORE_COST


def _sum_products(m, extra=None):
    def plus(a, b):
        return [add(u, v) for u, v in zip(a, b)]

    c00, both = (yield from m(1)), (yield from m(2))
    c00, c01 = plus(c00, both), (plus((yield from extra(0)), both) if extra else both)
    c11, both = (yield from m(3)), (yield from m(4))
    c11, c10 = plus(c11, both), (plus((yield from extra(1)), both) if extra else both)
    diag = yield from m(0)
    c00, c11 = plus(c00, diag), [sub(u, v) for u, v in zip(c11, diag)]
    both = (yield from extra(2)) if extra else None
    col = yield from m(5)
    col = plus(col, both) if extra else col
    c00, c10 = plus(c00, col), plus(c10, col)
    col = yield from m(6)
    col = plus(col, both) if extra else col
    return [c00, plus(c01, col), c10, plus(c11, col)]


def _contract(get):
    def inner(p):
        def leaf(n):
            yield 2
            return [get(7 * p + n)]
        return [v[0] for v in (yield from _sum_products(leaf))]

    out = yield from _sum_products(inner)
    return {(2 * (a // 2) + b // 2, 2 * (a % 2) + b % 2): out[a][b] for a in range(4) for b in range(4)}


def _slab(op, blk):
    return blk(op) if op < 2 else sub(blk(op - 2), blk(3 - op))


def _left_operand(n, w):
    def slab(use, tiles):
        return _slab(use[1], lambda i: w(i, tiles[use[0]]))

    p, e = divmod(n, 2) if n < 14 else (n - 7, 0) if n < 17 else (0, 2)
    if p >= 7:
        low, high = slab(A_SLABS[p][0], (4, 5)), slab(A_SLABS[p][1], (2, 3, 4))
    elif e == 0:
        return _combine(A_TERMS[p], w)
    else:
        low = _combine(A_TERMS[p], lambda i, k: w(i, 2 + k))
        high = slab(A_SLABS[p], (2, 3, 4)) if p else _combine(A_TERMS[p], w)
        if n == 1:
            high = pltpu.roll(high, T // 2, 1)
    return lax.select(lax.broadcasted_iota(jnp.int32, low.shape, 1) < T // 2, low, high)


def _right_operand(n, t, h):
    def slab(use):
        return _slab(use[1], lambda j: h(SLAB_ROW[use[0]] // 16 + t % 4, j))

    p, e = divmod(n, 2)
    if n >= 14:
        return slab(B_SLABS[n - 7][t // 4])
    if e == 0 or t < 4:
        return _combine(B_TERMS[p], lambda k, j: h(16 * e + 8 * k + t, j))
    return slab(B_SLABS[p])


def _chain(streams):
    def gen():
        for g, _ in streams:
            yield from g
    return gen(), sum(c for _, c in streams)


def _merge(lists, run=1):
    def gen():
        live = [[*_chain(streams), 0.0] for streams in lists]
        while live:
            s = min(live, key=lambda z: z[2] / z[1])
            for _ in range(run):
                cost = next(s[0], None)
                if cost is None:
                    live.remove(s)
                    break
                s[2] += cost
                yield cost
    return gen(), sum(c for streams in lists for _, c in streams)


def _trace(*lists):
    for _ in _merge(lists)[0]:
        pass


def _in_turns(*lists):
    keyed = [((n + 0.5) / len(streams), k, v) for k, streams in enumerate(lists) for n, v in enumerate(streams)]
    return [v for _, _, v in sorted(keyed, key=lambda z: z[:2])]


def _pieces(fn, *args, lo=0, hi=8):
    return [fn(*args, t, t + 1) for t in range(lo, hi)]


def _call(fn, *args):
    def gen():
        fn(*args)
        yield 1
    return gen(), 1


def _idle(cost):
    return iter([cost]), cost


def _kernel(x_hbm, wqkv_hbm, wo_hbm, w1_hbm, b1_hbm, w2_hbm, b2_hbm, c_hbm, wm_hbm, o_hbm,
            XB, WM, WQ, WO, W1R, W2R, WS, B1V, B2V, CV, B1, SB, V0, ROW, MOD, WP, WOP, MIX, H1, STAT, TT,
            OB, X1, HB, WL, WT, BC, W1, W2, M1, Z, GB, ACC, flag, sem, wsem):
    SA, CA, GA, SB2, CB, GB2, B2 = (i * D for i in range(7))
    OUT = WM
    TURN, QKV = M1
    traced = []

    def qkv_rows(tile, row, n=8):
        return _rows(0, n, tile * 3 * D + row)

    def product_rows(p, row=0, n=T):
        return _rows(0, n, p * (T + 8) + row)

    def cols(src, dst, lo, hi):
        return src.at[:, lo:hi], dst.at[:, lo:hi]

    moves = dict(
        c=(c_hbm, CV), b1=(b1_hbm, B1V), b2=(b2_hbm, B2V), wo=(wo_hbm, WO),
        **{f'wm{n}': cols(wm_hbm, WM, lo * T, hi * T)
           for n, (lo, hi) in enumerate(((0, 3), (3, 6), (6, 9), (9, 24), (24, 27)))},
        **{k: cols(wqkv_hbm, WQ, lo * T, min(hi * T, 3 * D))
           for k, lo, hi in (('wq0', 0, 2), ('wq1', 2, 4), ('wk0', 4, 7), ('wk1', 7, 9), ('wv', 9, 14))},
        **{f'ws{n}': (w1_hbm.at[_rows(n, 64), _rows(n, FC)], WS.at[_rows(n, 64)]) for n in range(8)},
        **{f'x{n}': (x_hbm.at[:, _rows(n, T)], XB.at[n]) for n in range(4 * NQ)},
        **{f'out{q}': cols(OUT, o_hbm, q * FC, (q + 1) * FC) for q in range(NQ - 1)},
        **{f'out3{d}': tuple(r.at[LAST[d] if d > 1 else 0:LAST[d + 1], S - FC:S] for r in (OUT, o_hbm))
           for d in (1, 2, 3)})
    copies = {k: pltpu.make_async_copy(s, d, sem.at[i]) for i, (k, (s, d)) in enumerate(moves.items())}

    def start(*names):
        for k in names:
            copies[k].start()

    def wait(*names):
        for k in names:
            copies[k].wait()

    def chunk(n, j, s):
        src, dst = ((w1_hbm, W1R), (w2_hbm, W2R))[n]
        return pltpu.make_async_copy(src.at[:, pl.ds(pl.multiple_of(j * FC, FC), FC)], dst.at[s], wsem.at[2 * n + s])

    def x_tiles(q):
        return [f'x{n}' for n in range(4 * q, 4 * q + 4)]

    def to_columns(row):
        return jnp.broadcast_to(row, (T, T)).T

    def silu_c():
        c = CV[...].astype(f32)
        s = _cat([c / (1.0 + jnp.exp(-c)), jnp.zeros((1, 5 * T - D), f32)], 1)
        for k in range(5):
            SB[_rows(k, T), :] = to_columns(s[:, _rows(k, T)])

    def mod(lo, hi):
        def gen():
            for j0 in range(lo, hi, 3):
                acc = [None] * 3
                for t in range(D // 16):
                    s = SB[_rows(t), :]
                    for u in range(3):
                        v = mul(_cast(WM[_rows(t), _rows(j0 + u, T)], f32), s)
                        acc[u] = v if t == 0 else add(acc[u], v)
                    yield 18
                for u in range(3):
                    row = jnp.sum(acc[u], axis=0, keepdims=True)
                    n = (j0 + u) * T + lax.broadcasted_iota(jnp.int32, (1, T), 1)
                    is_scale = ((n >= CA) & (n < CA + D)) | ((n >= CB) & (n < CB + D))
                    row = jnp.where(is_scale, 1.0 + row, row)
                    row = row * jnp.where(n >= GB2, 0.5 / GS, jnp.where(n >= SB2, GS, 1.0))
                    ROW[j0 + u] = jnp.broadcast_to(row, (8, T))
                    traced.append(j0 + u)
        return gen(), (hi - lo) * 6 * (D // 16)

    def biases():
        B1[...] = GS * B1V[...].astype(f32).reshape(1, F)
        b = 2.0 * GS * _cat([B2V[...].astype(f32).reshape(1, D), jnp.zeros((1, 5 * T - D), f32)], 1)
        for k in range(5):
            ROW[B2 // T + k] = jnp.broadcast_to(b[:, _rows(k, T)], (8, T))
            traced.append(B2 // T + k)

    def columns(lo, hi):
        def gen():
            for j in range(lo, hi):
                assert j in traced
                MOD[_rows(j, T), :] = _cat([ROW[j]] * (T // 8)).T
                yield 30
        return gen(), 30 * (hi - lo)

    def whole_tile(v):
        return v if v.shape[1] == T else _cat([v, jnp.zeros_like(v)], 1)

    def head_rows(k, base, d):
        return _cat(TURN[k % 4][pl.ds(k // 4 * 14 * T + base + d + e, 8, stride=DH), :] for e in range(2))

    def wqkv_transpose(lo, hi):
        def gen():
            for j in range(lo, hi):
                for k, halves in enumerate(DEPTH_TILES):
                    v = _cat(WQ[r:r + 64, j * T:min((j + 1) * T, 3 * D)] for r in halves).astype(f32)
                    TURN[k % 4][_rows(k // 4 * 14 + j, T), :] = whole_tile(v).T
                    yield 32
        return gen(), (hi - lo) * 6 * 32

    def wqkv_expand(m, g):
        def gen():
            for d in range(0, DH, 2):
                w = _once(lambda i, k: head_rows(k, m * D + (2 * g + i) * DB, d))
                for n in range(18):
                    WP[2 * m + g, n, _rows(d // 2), :] = _cast(_left_operand(n, w), bf16)
                    yield 4
            traced.append((m, g))
        return gen(), 9 * 18 * 4

    def wo_stage():
        def gen():
            for j in range(5):
                for k in range(D // 64):
                    v = WO[_rows(k, 64), j * T:min((j + 1) * T, D)].astype(f32)
                    TURN[j % 4][_rows(j // 4 * 28 + k, 64), :] = whole_tile(v)
                    yield 8
        return gen(), 45 * 8

    def wo_transpose():
        def gen():
            for j in range(5):
                parts = [head_rows(j, g * DB, d) for g in range(4) for d in range(0, DH, 2)]
                a, b, c = parts[24:28], parts[28:32], parts[32:36]
                parts = parts[:24] + a + c + a + b + b + c
                for k in range(6):
                    v = _cat(parts[8 * k:8 * k + 8]).T.astype(bf16)
                    for r in range(j * T, min((j + 1) * T, D), 16):
                        WOP[r // DB, k, _rows(0, 16, r % DB), :] = v[_rows(0, 16, r % T)]
                    yield 40
        return gen(), 30 * 40

    lane = lax.broadcasted_iota(jnp.int32, (8, T), 1)
    quarter = lane // 32

    def by_quarter(v):
        even, low = quarter % 2 == 0, quarter < 2
        half = [lax.select(even, v[-i % 4], v[(1 - i) % 4]) for i in range(4)]
        return [lax.select(low, half[i], half[(i + 2) % 4]) for i in range(4)]

    def deal_within(q):
        def gen():
            for s in range(4):
                src = (lane % 32 // 2) * 8 + ((quarter + 4 - s) % 4) * 2 + lane % 2
                for t in range(D // 16):
                    TT[q, s, _rows(t, 8), :] = jnp.take_along_axis(XB.bitcast(u32)[4 * q + s, _rows(t, 8), :], src, axis=1)
                    yield 2
        return gen(), 8 * 36

    def deal_across(q):
        def gen():
            for t in range(D // 16):
                for i, u in enumerate(by_quarter([TT[q, s, _rows(t, 8), :] for s in range(4)])):
                    MIX[4 * q + i, _rows(t, 8), :] = pltpu.roll(u, T - 32 * i, 1) if i else u
                yield 12
        return gen(), 12 * 36

    def collect_across(q, t):
        v = [XB.bitcast(u32)[4 * q + i, _rows(t, 8), :] for i in range(4)]
        for s, u in enumerate(by_quarter([pltpu.roll(v[i], 32 * i, 1) if i else v[0] for i in range(4)])):
            TT[q, s, _rows(t, 8), :] = u

    def collect_within(q, lo=0, hi=D // 16):
        def gen():
            for s in range(4):
                src = ((lane % 8 // 2 + s) % 4) * 32 + (lane // 8) * 2 + lane % 2
                for t in range(lo, hi):
                    u = jnp.take_along_axis(TT[q, s, _rows(t, 8), :], src, axis=1)
                    OUT[_rows(t), _rows(4 * q + s, T)] = pltpu.bitcast(u, bf16)
                    yield 2
        return gen(), (hi - lo) * 8

    def dealt(tile, t):
        return _cast(pltpu.bitcast(MIX[tile, _rows(t, 8), :], bf16), f32)

    def moments(tile, load, cost):
        for t in range(D // 16):
            v = load(t)
            if t == 0:
                pivot = jnp.broadcast_to(jnp.sum(v, axis=0, keepdims=True) * (1.0 / 16), (16, T))
            dv = sub(v, pivot)
            s1, s2 = (dv, mul(dv, dv)) if t == 0 else (add(s1, dv), add(s2, mul(dv, dv)))
            yield cost
        m1 = jnp.sum(s1, axis=0, keepdims=True) * (1.0 / D)
        m2 = jnp.sum(s2, axis=0, keepdims=True) * (1.0 / D)
        STAT[tile, 0] = pivot[:8] + m1
        STAT[tile, 1] = jnp.broadcast_to(lax.rsqrt(jnp.maximum(m2 - m1 * m1, 0.0) + EPS), (8, T))

    def normaliser():
        stat = _once(lambda tile, k: _cat([STAT[tile, k]] * 2))
        return lambda v, tile: mul(sub(v, stat(tile, 0)), stat(tile, 1))

    def modulate(v, t, scale, shift):
        return add(mul(v, MOD[_rows(t, 16, scale), :]), MOD[_rows(t, 16, shift), :])

    def ln1_moments(q):
        def gen():
            for tile in range(4 * q, 4 * q + 4):
                yield from moments(tile, lambda t: dealt(tile, t), 10)
        return gen(), 4 * 36 * 10

    def ln1_scale(q):
        normalise = normaliser()
        for i in range(4):
            for t in range(D // 16):
                X1[q][i, _rows(t), :] = normalise(dealt(4 * q + i, t), 4 * q + i)

    def ln1_apply(q, scaled=False):
        def gen():
            normalise = normaliser()

            def put(i, n, t, v):
                H1[2 * q + i, n, _rows(t), :] = _cast(v, bf16)

            def load(i, n):
                v = X1[q][i, _rows(n), :] if scaled else normalise(dealt(4 * q + i, n), 4 * q + i)
                return modulate(v, n, CA, SA)

            for t in range(8):
                first = []
                for i in range(2):
                    h = _once(lambda n, j: load(2 * i + j, n))
                    first.append([_right_operand(n, t, h) for n in range(2 if t < 4 else 1)])
                    for n in range(2, 14):
                        put(i, n, t, _right_operand(n, t, h))
                        yield 12
                    for n in range(14, 17 if t >= 4 else 0):
                        for u in (t - 4, t):
                            put(i, n, u, _right_operand(n, u, h))
                if t < 4:
                    put(0, 0, t, first[0][0])
                    put(1, 1, 4 + t, first[1][0])
                    put(0, 1, t, first[0][1])
                    put(1, 1, t, sub(first[1][1], first[0][1]))
                else:
                    put(0, 1, t, first[1][0])
                    put(0, 0, t, sub(first[0][0], first[1][0]))
        return gen(), 2 * 8 * 12 * 12

    def ln2_moments(q):
        def gen():
            for i in range(4):
                def residual(t):
                    v = add(dealt(4 * q + i, t), mul(MOD[_rows(t, 16, GA), :], X1[q][i, _rows(t), :]))
                    X1[q][i, _rows(t), :] = v
                    return v
                yield from moments(4 * q + i, residual, 14)
            traced.append(('ln2', q))
        return gen(), 4 * 36 * 14

    def ln2_apply(q):
        def gen():
            assert ('ln2', q) in traced
            normalise = normaliser()
            for t in range(9):
                blk = {}
                for k in range(4):
                    for i in range(4):
                        blk[k, i] = modulate(normalise(X1[q][i, _rows(4 * t + k), :], 4 * q + i), 4 * t + k, CB, SB2)
                        if t == 8:
                            HB[q][NP + i, _rows(k), :] = _cast(blk[k, i], bf16)
                        yield 8

                def emit(p, v):
                    HB[q][p, _rows(t), :] = v
                yield from _expand(B_TERMS, blk, emit)
        return gen(), 9 * (128 + EXPAND_COST)

    def project(q, m, pairs=(0, 1)):
        def gen():
            for g in pairs:
                assert (m, g) in traced
                both = _dot(_ld(WP, 2 * m + g, 17), _ld(H1, 2 * q, 1))
                yield DB
                for i in range(2):
                    def part(tiles, acc=None):
                        for n in tiles:
                            v = _dot(_ld(WP, 2 * m + g, n), _ld(H1, 2 * q + i, n))
                            acc = v if acc is None else add(acc, v)
                            yield DB
                        return [acc]
                    out = yield from _sum_products(lambda p: part((2 * p, 2 * p + 1)) if p else part((i,), both),
                                                   lambda p: part((14 + p,)))
                    for n, (v,) in enumerate(out):
                        QKV[q][qkv_rows(2 * i + n % 2, m * D + (2 * g + n // 2) * DB, DB), :] = v
        return gen(), len(pairs) * 33 * DB

    def first_value():
        def gen():
            for row in range(0, D, 8):
                V0[row:row + 8, :] = jnp.take_along_axis(QKV[0][qkv_rows(0, 2 * D + row), :], lane * 0, axis=1)
                yield 2
        return gen(), D // 4

    def attend(q):
        logit, prob = {}, {}
        from_lane = _once(lambda n: lane >= n)

        def tile(row, j):
            back = -2 * (j // 4)
            v = QKV[q][qkv_rows(j % 4, row), :]
            if back and q:
                v = lax.select(from_lane(T - back), QKV[q - 1][qkv_rows(j % 4, row), :], v)
            if back:
                v = pltpu.roll(v, back, 1)
            if back and not q and row >= 2 * D:
                v = lax.select(from_lane(back), v, V0[_rows(0, 8, row - 2 * D), :])
            return v

        def users(j):
            return [i for i in range(4) if 0 <= i - j < WIN]

        def score(g):
            def gen():
                for js in ((3, 0, -1, -4, -7), (2, 1, -2, -3, -5, -6)):
                    for d in range(DH):
                        row = g * DB + d * 8
                        query = _once(lambda i: tile(row, i))
                        for j in js:
                            k = tile(D + row, j)
                            for i in users(j):
                                u = mul(query(i), k)
                                logit[i, j] = u if d == 0 else add(logit[i, j], u)
                            yield 2 * len(users(j))
            return gen(), DH * 64

        def softmax(g):
            def gen():
                for i in range(4):
                    js = [i - w for w in range(WIN)]
                    z = [logit[i, j] * (SCALE * LOG2E) for j in js]
                    if q == 0:
                        z = [jnp.where(from_lane(-2 * (j // 4)), u, -1e9 * LOG2E) if j < 0 else u
                             for j, u in zip(js, z)]
                    top = z[0]
                    for u in z[1:]:
                        top = lax.max(top, u)
                    e = [lax.exp2(sub(u, top)) for u in z]
                    inv = 1.0 / (((e[0] + e[1]) + (e[2] + e[3])) + ((e[4] + e[5]) + (e[6] + e[7])))
                    for j, u in zip(js, e):
                        prob[i, j] = mul(u, inv)
                    yield 50
            return gen(), 200

        def mix(g):
            def gen():
                for row in range(g * DB, (g + 1) * DB, 16):
                    o = {}
                    for j in (3, -1, -2, 2, -3, -4, 1, -5, -6, 0, -7):
                        v = [tile(2 * D + row + h, j) for h in (0, 8)]
                        for i in users(j):
                            for h in range(2):
                                u = mul(prob[i, j], v[h])
                                o[i, h] = add(o[i, h], u) if (i, h) in o else u
                        yield 4 * len(users(j))
                    for n in range(2):
                        u, v = (_cat([o[i, 0], o[i, 1]]) for i in (2 * n, 2 * n + 1))
                        slab, r = divmod(row, 64)
                        if slab < 7:
                            put = ((row, u), (4 * T + row, v))
                        elif slab == 7:
                            put = ((8 * T + r, u), (4 * T + row, sub(v, u)))
                        else:
                            put = ((7 * 64 + r, sub(u, v)), (8 * T + 64 + r, v))
                        for r, w in put:
                            OB[2 * q + n, r:r + 16, :] = _cast(w, bf16)
            return gen(), DH * 64

        return _chain([f(g) for g in range(4) for f in (score, softmax, mix)])

    def project_out(q):
        def gen():
            for g in range(4):
                for n in range(2):
                    both = _dot(_ld(WOP, g, 5), _ld(OB, 2 * q + n, _rows(8, T // 2)))
                    yield DB
                    for i in range(2):
                        acc = both
                        for k in range(4):
                            w = _ld(WOP, g, k if k < 3 else 3 + i)
                            acc = add(acc, _dot(w, _ld(OB, 2 * q + n, _rows(4 * i + k, T // 2))))
                            if k == 3:
                                X1[q][2 * n + i, _rows(g, DB), :] = acc
                            yield DB
        return gen(), 72 * DB

    def slabs(j, among, load):
        if isinstance(j, int):
            return [load(8 if j == t else t) for t in range(8)]
        return [jnp.where(j == t, load(8), load(t)) if t in among else load(t) for t in range(8)]

    def is_chunk(j, n):
        return isinstance(j, int) and j == n

    def w1_transpose(j, s):
        def gen():
            for i in range(4):
                for k in range(4):
                    def load(n):
                        at = _rows(4 * n + k), _rows(i, T)
                        if is_chunk(j, SHARED):
                            return _cast(WS[at], f32)
                        v = _cast(W1R[(s, *at)], f32)
                        return v if n == 8 else sub(v, _cast(WS[at], f32))
                    WT[s, i, k, 0:T, :] = _cat(slabs(j, range(6 - s, 8, 2), load)).T
                    yield 64
        return gen(), 16 * 64

    def w1_last_slab():
        for i in range(4):
            v = W1R[(NC - 1) % 2, 4 * T:D, _rows(i, T)]
            WL[i] = _cat([v, jnp.zeros_like(v)]).T

    def w1_expand(j, s, lo=0, hi=8):
        def gen():
            for t in range(lo, hi):
                def emit(p, v):
                    W1[s][p, _rows(t), :] = v
                yield from _expand(A_TERMS, {(i, k): WT[s, i, k, _rows(t), :] for i in range(4) for k in range(4)}, emit)
                if t % 2 and not is_chunk(j, SHARED):
                    BC[s, t // 2] = to_columns(B1[:, pl.ds(pl.multiple_of(j * FC + t // 2 * T, T), T)])
            traced.append(('w1', s))
        return gen(), (hi - lo) * EXPAND_COST

    def w2_expand(s, lo, hi):
        def gen():
            for t in range(lo, hi):
                blk = {}
                for d in range(4):
                    for k in range(4):
                        blk[d, k] = _cast(W2R[s, _rows(4 * t + d), _rows(k, T)], f32)
                        yield 2

                def emit(p, v):
                    W2[s][p, _rows(t), :] = v
                yield from _expand(A_TERMS, blk, emit)
        return gen(), (hi - lo) * (32 + EXPAND_COST)

    def up(j, s, q):
        extra = 16 if is_chunk(j, NC - 1) else 0

        def gen():
            assert ('w1', s) in traced
            words = HB[q].bitcast(u32)
            for p in range(NP):
                h = _cat(slabs(j, range(4 - s, 8, 2), _once(lambda n: words[p, _rows(n, 8), :])))
                v = _dot(_ld(W1[s], p), pltpu.bitcast(h, bf16))
                if p in ROW_PRODUCTS and not is_chunk(j, SHARED):
                    v = add(v, BC[s, ROW_PRODUCTS.index(p)])
                M1[s][q][product_rows(p), :] = v
                yield T
            for n in range(extra):
                M1[s][q][product_rows(NP + n), :] = _dot(_ld(WL, n // 4), _ld(HB[q], NP + n % 4, slice(0, T // 2)))
                yield T
        return gen(), (NP + extra) * T

    def keep_shared(q):
        def gen():
            for r in range(0, T, 8):
                z = yield from _contract(lambda p: M1[1][q][product_rows(p, r, 8), :])
                for (c, i), v in z.items():
                    Z[q][product_rows(4 * c + i, r, 8), :] = v
                    yield 1
        return gen(), 16 * (2 * NP + 16)

    def activate(j, s, q, lo=0, hi=8):
        rest, at = (M1[s][q], NP) if is_chunk(j, NC - 1) else (Z[q], 0)
        plain = is_chunk(j, NC - 1) and q == NQ - 1

        def gen():
            for t in range(lo, hi):
                halves = []
                for r in (16 * t, 16 * t + 8):
                    pre = yield from _contract(lambda p: M1[s][q][product_rows(p, r, 8), :])
                    for (c, i), u in pre.items():
                        u = add(u, rest[product_rows(at + 4 * c + i, r, 8), :])
                        pre[c, i] = add(mul(u, lax.tanh(mul(u, add(mul(u, u), GK)))), u)
                        yield GELU_COST
                    halves.append(pre)
                blk = {k: _cat([halves[0][k], halves[1][k]]) for k in halves[0]}

                def emit(p, v):
                    GB[s][q][p, _rows(t), :] = v
                if plain:
                    for (c, i), v in blk.items():
                        emit(4 * c + i, _cast(v, bf16))
                else:
                    yield from _expand(B_TERMS, blk, emit)
        return gen(), (hi - lo) * (4 * NP + 32 * GELU_COST + (0 if plain else EXPAND_COST))

    def down(s, q, first=False):
        def gen():
            for p in range(NP):
                v = _dot(_ld(W2[s], p), _ld(GB[s][q], p))
                if not first:
                    v = add(v, ACC[q][p])
                elif p in ROW_PRODUCTS:
                    v = add(v, _cat(MOD[_rows(n, 16, B2), :] for n in range(ROW_PRODUCTS.index(p), D // 16, 4)))
                ACC[q][p] = v
                yield DB
        return gen(), NP * DB

    def finish(q, lo=0, hi=DB // 16):
        def gen():
            for t in range(lo, hi):
                halves = []
                for r in (_rows(2 * t, 8), _rows(2 * t + 1, 8)):
                    halves.append((yield from _contract(lambda p: ACC[q][p, r, :])))
                done = q < NQ - 1 or 64 * t < LAST[2]
                for d in range(4):
                    r = _rows(4 * t + d)
                    gate = MOD[_rows(4 * t + d, 16, GB2), :]
                    for i in range(4):
                        y = add(X1[q][i, r, :], mul(gate, _cat([halves[0][d, i], halves[1][d, i]])))
                        if done:
                            XB[4 * q + i, r, :] = _cast(y, bf16)
                        else:
                            X1[q][i, r, :] = y
                        yield 5
                    if done:
                        collect_across(q, 4 * t + d)
                    yield 12
        return gen(), (hi - lo) * (4 * NP + 16 * 5 + 48)

    def down_last(d):
        q, s, (lo, hi) = NQ - 1, (NC - 1) % 2, LAST[d:d + 2]

        def gen():
            for i in range(4):
                for k in range(4):
                    v = _dot(W2R[s, lo:hi, _rows(k, T)], _ld(GB[s][q], 4 * k + i))
                    acc = v if k == 0 else add(acc, v)
                    yield hi - lo
                y = add(X1[q][i, lo:hi, :], mul(MOD[GB2 + lo:GB2 + hi, :], acc))
                if d < 2:
                    X1[q][i, lo:hi, :] = y
                else:
                    XB[4 * q + i, lo:hi, :] = _cast(y, bf16)
            traced.append(('last', d))
        return gen(), 16 * (hi - lo)

    def send_last(d):
        assert ('last', d) in traced
        for t in range(LAST[d] // 16, LAST[d + 1] // 16):
            collect_across(NQ - 1, t)
        _trace([collect_within(NQ - 1, LAST[d] // 16, LAST[d + 1] // 16)])
        start(f'out3{d}')

    start('c', *x_tiles(0), 'wk0', 'wm0', 'wm1', 'wm2', 'wk1')

    @pl.loop(0, 4)
    def _(n):
        flag[0] = n

    for q in range(NQ):
        HB[q][NP:, 64:T, :] = jnp.zeros((4, 64, T), bf16)

    def block(*lists):
        pl.when(flag[0] >= 0)(lambda: _trace(*lists))

    def ln1(q):
        return [ln1_moments(q), ln1_apply(q)]

    def activate_all(j, s, groups=range(NQ)):
        return [v for q in groups for v in _pieces(activate, j, s, q)]

    shared = [f'ws{n}' for n in range(8)]
    wait('c')
    silu_c()
    wait(*x_tiles(0))
    block([deal_within(0), deal_across(0)])
    wait('wk0')
    block([wqkv_transpose(4, 7), wqkv_expand(1, 0)], [ln1_moments(0)])
    block([_call(ln1_scale, 0)])
    wait('wm0', 'wm1')
    start('wq1', 'wq0')
    block([mod(0, 6), columns(0, 6)])
    wait('wm2')
    start(*x_tiles(1), 'wv')
    block([mod(6, 9), columns(6, 9), ln1_apply(0, True)])
    wait('wk1')
    block([project(0, 1, (0,))], [wqkv_transpose(7, 9), wqkv_expand(1, 1)])
    wait('wq1')
    block([project(0, 1, (1,))], [wqkv_transpose(2, 4), wqkv_expand(0, 1)])
    wait('wq0', *x_tiles(1))
    start(*x_tiles(2))
    block([project(0, 0, (1,))], [wqkv_transpose(0, 2), wqkv_expand(0, 0)], [deal_within(1)])
    wait('wv')
    start(*x_tiles(3))
    block([project(0, 0, (0,))], [wqkv_transpose(9, 14), wqkv_expand(2, 0), deal_across(1)])
    wait(*x_tiles(2))
    start('wo', 'b1', 'b2')
    block([project(0, 2)], [wqkv_expand(2, 1)] + ln1(1), [deal_within(2), deal_across(2)])
    wait(*x_tiles(3), 'wo', 'b1', 'b2')
    block([project(1, 1)], ln1(2), [deal_within(3), first_value(), deal_across(3)], [wo_stage(), _call(biases)])
    block([project(1, 0), project(1, 2), project(2, 1)], [attend(0), wo_transpose()],
          [ln1_moments(3), _call(start, 'wm3', *shared), ln1_apply(3)])
    wait('wm3', *shared)
    chunk(0, 0, 0).start()
    block([project(2, 0), project(2, 2), project_out(0)], [attend(1), w1_transpose(SHARED, 1), columns(9, 24)],
          [mod(9, 24), _idle(900)])
    chunk(0, 0, 0).wait()
    chunk(0, 1, 1).start()
    block([project(3, 0), project(3, 1), project(3, 2), project_out(1)],
          [attend(2), w1_expand(SHARED, 1), ln2_apply(0)], [ln2_moments(0), w1_transpose(0, 0)])
    chunk(1, 0, 0).start()
    chunk(0, 2, 0).start()
    block([project_out(2), up(SHARED, 1, 0), up(0, 0, 0)], [w1_expand(0, 0), attend(3)], [ln2_moments(1)])
    chunk(1, 1, 1).start()
    block([project_out(3)], [ln2_apply(1), ln2_moments(2)], [columns(27, 32)])
    block([up(SHARED, 1, 1), up(0, 0, 1)], [ln2_moments(3), keep_shared(0), ln2_apply(2), ln2_apply(3)])
    chunk(0, 1, 1).wait()
    chunk(1, 0, 0).wait()
    block([up(SHARED, 1, 2), up(SHARED, 1, 3), up(0, 0, 2), up(0, 0, 3)],
          [keep_shared(1)] + _in_turns(activate_all(0, 0, (0, 1)), _pieces(w2_expand, 0, hi=9)), [w1_transpose(1, 1)])
    chunk(0, 3, 1).start()
    chunk(1, 2, 0).start()
    chunk(0, 2, 0).wait()
    block([down(0, 0, True), down(0, 1, True)], [keep_shared(2), w1_expand(1, 1), keep_shared(3)], [w1_transpose(2, 0)])
    chunk(0, 4, 0).start()
    chunk(0, 3, 1).wait()
    chunk(1, 1, 1).wait()
    block([up(1, 1, q) for q in range(NQ)],
          _in_turns(activate_all(0, 0, (2, 3)), _pieces(w1_expand, 2, 0) + _pieces(w2_expand, 1, hi=5)), [w1_transpose(3, 1)])
    chunk(0, 5, 1).start()
    chunk(0, 4, 0).wait()
    start('wm4')
    block([_merge([[up(2, 0, q) for q in range(NQ)], [down(0, 2, True), down(0, 3, True)]], 3)],
          _in_turns(activate_all(1, 1), _pieces(w2_expand, 1, lo=5, hi=9) + _pieces(w1_expand, 3, 1)), [w1_transpose(4, 0)])

    def step(j, s):
        chunk(0, jnp.minimum(j + 3, NC - 1), 1 - s).wait()
        chunk(1, j, s).wait()
        pl.when(j < NC - 3)(lambda: chunk(0, jnp.minimum(j + 4, NC - 1), s).start())
        chunk(1, j + 1, 1 - s).start()
        if s == 1:
            @pl.when(j + 3 == NC - 1)
            def _():
                WS[...] = jnp.zeros(WS.shape, bf16)
        block([_merge([[up(j + 1, 1 - s, q) for q in range(NQ)], [down(1 - s, q) for q in range(NQ)]], RUN)],
              _in_turns(activate_all(j, s), _pieces(w2_expand, s, hi=9) + _pieces(w1_expand, j + 2, s)),
              [w1_transpose(j + 3, 1 - s)] + [_call(w1_last_slab)] * s)

    @pl.loop(1, NC // 2)
    def _(n):
        step(2 * n, 0)
        pl.when(n < NC // 2 - 1)(lambda: step(2 * n + 1, 1))

    chunk(1, 7, 1).wait()
    wait('wm4')
    chunk(1, 8, 0).start()
    block([_merge([[up(8, 0, 0), up(8, 0, 1)], [down(0, q) for q in range(NQ)]], 3)],
          _in_turns(activate_all(7, 1)[:-3], _pieces(w2_expand, 1, hi=9)), [mod(24, 27)])
    chunk(1, 8, 0).wait()
    block([_merge([[up(8, 0, 2), up(8, 0, 3)], [down(1, 0)]], 4)],
          _in_turns(activate_all(8, 0, (0, 1)), _pieces(w2_expand, 0, hi=9)))
    block([down(0, 0), down(1, 1)], [activate(8, 0, 2), activate(7, 1, 3, 5, 8)], [columns(24, 27)])
    block([down(0, 1), down(1, 2)], _in_turns(activate_all(8, 0, (3,)), _pieces(finish, 0, hi=9)))
    block([down(0, 2)], [finish(1)], [collect_within(0)])
    start('out0')
    block([down(1, 3)], [finish(2)], [collect_within(1)])
    start('out1')
    block([down_last(0), down_last(1)], [finish(3, 4, 9)], [collect_within(2)])
    start('out2')
    block([down_last(2), down_last(3)],
          [finish(3, 0, 4), collect_within(3, 0, 16), _call(start, 'out31'), _call(send_last, 2), _idle(400)])
    block([_call(send_last, 3)])
    wait(*[k for k in copies if k.startswith('out')])


@jax.jit
def pallas_adaLN_cond__sliding_local_dilated__dense_activation_gelu__prompt_kernel(
    A_x: jax.Array,
    A_wqkv: jax.Array,
    A_wo: jax.Array,
    B_x: jax.Array,
    B_w1: jax.Array,
    B_b1: jax.Array,
    B_w2: jax.Array,
    B_b2: jax.Array,
    c: jax.Array,
    w_mod: jax.Array,
):
    del B_x
    assert A_x.shape == (1, S, D) and B_w1.shape == (D, F)
    vmem = pltpu.VMEM
    scratch = [
        vmem((4 * NQ, D, T), bf16),
        vmem((D, 6 * D), bf16),
        vmem((D, 3 * D), bf16),
        vmem((D, D), bf16),
        vmem((2, D, FC), bf16),
        vmem((2, D, FC), bf16),
        vmem((4 * T, FC), bf16),
        vmem((F,), bf16), vmem((D,), bf16), vmem((1, D), bf16),
        vmem((1, F), f32),
        vmem((5 * T, T), f32),
        vmem((D, T), f32),
        vmem((32, 8, T), f32),
        vmem((32 * T, T), f32),
        vmem((6, 18, DB, T), bf16),
        vmem((4, 6, DB, T), bf16),
        vmem((4 * NQ, D // 2, T), u32),
        vmem((2 * NQ, 17, T, T), bf16),
        vmem((4 * NQ, 2, 8, T), f32),
        vmem((NQ, 4, D // 2, T), u32),
        vmem((2 * NQ, 9 * T, T), bf16),
        [vmem((4, D, T), f32)] * NQ,
        [vmem((NP + 4, DB, T), bf16)] * NQ,
        vmem((4, T, T), bf16),
        vmem((2, 4, 4, T + 8, T), f32),
        vmem((2, 4, T, T), f32),
        [vmem((NP, T, T), bf16)] * 2,
        [vmem((NP, DB, T), bf16)] * 2,
        [[vmem(((NP + 16) * (T + 8), T), f32)] * NQ, [vmem((12 * D, T), f32)] * NQ],
        [vmem((16 * (T + 8), T), f32)] * NQ,
        [[vmem((NP, T, T), bf16)] * NQ] * 2,
        [vmem((NP, DB, T), f32)] * NQ,
        pltpu.SMEM((1,), jnp.int32),
        pltpu.SemaphoreType.DMA((44,)),
        pltpu.SemaphoreType.DMA((4,)),
    ]
    out = pl.pallas_call(
        _kernel,
        out_shape=jax.ShapeDtypeStruct((D, S), A_x.dtype),
        in_specs=[pl.BlockSpec(memory_space=pl.ANY)] * 9,
        out_specs=pl.BlockSpec(memory_space=pl.ANY),
        scratch_shapes=scratch,
        compiler_params=pltpu.CompilerParams(
            vmem_limit_bytes=124 * 2**20,
            flags={'XLA_TPU_EVENLY_DISTRIBUTE_CRITICAL_NODES': True}),
        name='adaln_block',
    )(A_x[0].T, A_wqkv, A_wo, B_w1, B_b1, B_w2.T, B_b2, c, w_mod)
    return out.T[None]
```

```python
import jax
import jax.numpy as jnp
import numpy as np
from jax import lax
from jax.experimental import pallas as pl
from jax.experimental.pallas import tpu as pltpu

f32, bf16, u32 = jnp.float32, jnp.bfloat16, jnp.uint32
add, sub, mul = lax.add, lax.sub, lax.mul

S, D, F = 2048, 576, 4608
DH, WIN = 18, 8
T = 128
NQ = 4
DB = D // 4
FC = 4 * T
NC = F // FC
NP = 49
SHARED = -1
LAST = (0, 128, 256, 416, 576)
EPS = 1e-5
LOG2E = float(np.log2(np.e))
SCALE = float(DH ** -0.5)
GS = float(np.cbrt(np.sqrt(2.0 / np.pi) * 0.044715))
GK = np.float32(np.sqrt(2.0 / np.pi) / GS)

A_TERMS = (((1, 0, 0), (1, 1, 1)), ((1, 0, 1), (-1, 1, 1)), ((1, 0, 0), (1, 0, 1)), ((1, 1, 0), (-1, 0, 0)),
           ((1, 1, 0), (1, 1, 1)), ((1, 1, 1),), ((1, 0, 0),))
B_TERMS = (((1, 0, 0), (-1, 1, 1)), ((1, 1, 0), (-1, 1, 1)), ((1, 1, 1),), ((1, 0, 1), (-1, 0, 0)),
           ((1, 0, 0),), ((1, 1, 0), (-1, 0, 0)), ((1, 0, 1), (-1, 1, 1)))
ROW_PRODUCTS = tuple(7 * a + b for a in (2, 4) for b in (2, 4))
A_SLABS = (None, (0, 0), (2, 2), (0, 1), (1, 3), (1, 0), (2, 1),
           ((0, 0), (2, 2)), ((0, 1), (1, 3)), ((1, 0), (2, 1)))
B_SLABS = (None, (0, 0), (2, 0), (0, 1), (1, 1), (1, 2), (2, 3),
           ((0, 1), (2, 3)), ((0, 0), (1, 2)), ((1, 1), (2, 0)))
SLAB_ROW = (320, 448, 512)
DEPTH_TILES = ((0, 64), (128, 192), (256, 320), (384, 448), (320, 512), (448, 512))

STORE_COST = 3
GELU_COST = 7
RUN = 7
EXPAND_COST = 2 * 55 + STORE_COST * NP


def _cast(v, dtype):
    return lax.convert_element_type(v, dtype)


def _cat(vals, axis=0):
    return lax.concatenate(list(vals), axis)


def _dot(a, b):
    return lax.dot_general(a, b, (((1,), (0,)), ((), ())), preferred_element_type=f32)


def _ld(ref, *idx):
    return pltpu.bitcast(ref.bitcast(u32)[idx], bf16)


def _rows(t, n=16, at=0):
    return slice(at + t * n, at + (t + 1) * n)


def _once(fn):
    kept = {}

    def get(*key):
        if key not in kept:
            kept[key] = fn(*key)
        return kept[key]
    return get


def _combine(term, blk):
    v = blk(*term[0][1:])
    for sign, r, c in term[1:]:
        v = (add if sign > 0 else sub)(v, blk(r, c))
    return v


def _expand(terms, blk, emit):
    for p, outer in enumerate(terms):
        part = {}
        for r in range(2):
            for c in range(2):
                part[r, c] = _combine(outer, lambda i, j: blk[2 * i + r, 2 * j + c])
                yield 2 * (len(outer) - 1)
        for n, inner in enumerate(terms):
            emit(7 * p + n, _cast(_combine(inner, lambda r, c: part[r, c]), bf16))
            yield 2 * (len(inner) - 1) + STORE_COST


def _sum_products(m, extra=None):
    def plus(a, b):
        return [add(u, v) for u, v in zip(a, b)]

    c00, both = (yield from m(1)), (yield from m(2))
    c00, c01 = plus(c00, both), (plus((yield from extra(0)), both) if extra else both)
    c11, both = (yield from m(3)), (yield from m(4))
    c11, c10 = plus(c11, both), (plus((yield from extra(1)), both) if extra else both)
    diag = yield from m(0)
    c00, c11 = plus(c00, diag), [sub(u, v) for u, v in zip(c11, diag)]
    both = (yield from extra(2)) if extra else None
    col = yield from m(5)
    col = plus(col, both) if extra else col
    c00, c10 = plus(c00, col), plus(c10, col)
    col = yield from m(6)
    col = plus(col, both) if extra else col
    return [c00, plus(c01, col), c10, plus(c11, col)]


def _contract(get):
    def inner(p):
        def leaf(n):
            yield 2
            return [get(7 * p + n)]
        return [v[0] for v in (yield from _sum_products(leaf))]

    out = yield from _sum_products(inner)
    return {(2 * (a // 2) + b // 2, 2 * (a % 2) + b % 2): out[a][b] for a in range(4) for b in range(4)}


def _slab(op, blk):
    return blk(op) if op < 2 else sub(blk(op - 2), blk(3 - op))


def _left_operand(n, w):
    def slab(use, tiles):
        return _slab(use[1], lambda i: w(i, tiles[use[0]]))

    p, e = divmod(n, 2) if n < 14 else (n - 7, 0) if n < 17 else (0, 2)
    if p >= 7:
        low, high = slab(A_SLABS[p][0], (4, 5)), slab(A_SLABS[p][1], (2, 3, 4))
    elif e == 0:
        return _combine(A_TERMS[p], w)
    else:
        low = _combine(A_TERMS[p], lambda i, k: w(i, 2 + k))
        high = slab(A_SLABS[p], (2, 3, 4)) if p else _combine(A_TERMS[p], w)
        if n == 1:
            high = pltpu.roll(high, T // 2, 1)
    return lax.select(lax.broadcasted_iota(jnp.int32, low.shape, 1) < T // 2, low, high)


def _right_operand(n, t, h):
    def slab(use):
        return _slab(use[1], lambda j: h(SLAB_ROW[use[0]] // 16 + t % 4, j))

    p, e = divmod(n, 2)
    if n >= 14:
        return slab(B_SLABS[n - 7][t // 4])
    if e == 0 or t < 4:
        return _combine(B_TERMS[p], lambda k, j: h(16 * e + 8 * k + t, j))
    return slab(B_SLABS[p])


def _chain(streams):
    def gen():
        for g, _ in streams:
            yield from g
    return gen(), sum(c for _, c in streams)


def _merge(lists, run=1):
    def gen():
        live = [[*_chain(streams), 0.0] for streams in lists]
        while live:
            s = min(live, key=lambda z: z[2] / z[1])
            for _ in range(run):
                cost = next(s[0], None)
                if cost is None:
                    live.remove(s)
                    break
                s[2] += cost
                yield cost
    return gen(), sum(c for streams in lists for _, c in streams)


def _trace(*lists):
    for _ in _merge(lists)[0]:
        pass


def _in_turns(*lists):
    keyed = [((n + 0.5) / len(streams), k, v) for k, streams in enumerate(lists) for n, v in enumerate(streams)]
    return [v for _, _, v in sorted(keyed, key=lambda z: z[:2])]


def _pieces(fn, *args, lo=0, hi=8):
    return [fn(*args, t, t + 1) for t in range(lo, hi)]


def _call(fn, *args):
    def gen():
        fn(*args)
        yield 1
    return gen(), 1


def _idle(cost):
    return iter([cost]), cost


def _kernel(x_hbm, wqkv_hbm, wo_hbm, w1_hbm, b1_hbm, w2_hbm, b2_hbm, c_hbm, wm_hbm, o_hbm,
            XB, WM, WQ, WO, W1R, W2R, WS, B1V, B2V, CV, B1, SB, V0, ROW, MOD, WP, WOP, MIX, H1, STAT, TT,
            OB, X1, HB, WL, WT, BC, W1, W2, M1, Z, GB, ACC, flag, sem, wsem):
    SA, CA, GA, SB2, CB, GB2, B2 = (i * D for i in range(7))
    OUT = WM
    TURN, QKV = M1
    traced = []

    def qkv_rows(tile, row, n=8):
        return _rows(0, n, tile * 3 * D + row)

    def product_rows(p, row=0, n=T):
        return _rows(0, n, p * (T + 8) + row)

    def cols(src, dst, lo, hi):
        return src.at[:, lo:hi], dst.at[:, lo:hi]

    moves = dict(
        c=(c_hbm, CV), b1=(b1_hbm, B1V), b2=(b2_hbm, B2V), wo=(wo_hbm, WO),
        **{f'wm{n}': cols(wm_hbm, WM, lo * T, hi * T)
           for n, (lo, hi) in enumerate(((0, 3), (3, 6), (6, 9), (9, 24), (24, 27)))},
        **{k: cols(wqkv_hbm, WQ, lo * T, min(hi * T, 3 * D))
           for k, lo, hi in (('wq0', 0, 2), ('wq1', 2, 4), ('wk0', 4, 7), ('wk1', 7, 9), ('wv', 9, 14))},
        **{f'ws{n}': (w1_hbm.at[_rows(n, 64), _rows(n, FC)], WS.at[_rows(n, 64)]) for n in range(8)},
        **{f'x{n}': (x_hbm.at[:, _rows(n, T)], XB.at[n]) for n in range(4 * NQ)},
        **{f'out{q}': cols(OUT, o_hbm, q * FC, (q + 1) * FC) for q in range(NQ - 1)},
        **{f'out3{d}': tuple(r.at[LAST[d] if d > 1 else 0:LAST[d + 1], S - FC:S] for r in (OUT, o_hbm))
           for d in (1, 2, 3)})
    copies = {k: pltpu.make_async_copy(s, d, sem.at[i]) for i, (k, (s, d)) in enumerate(moves.items())}

    def start(*names):
        for k in names:
            copies[k].start()

    def wait(*names):
        for k in names:
            copies[k].wait()

    def chunk(n, j, s):
        src, dst = ((w1_hbm, W1R), (w2_hbm, W2R))[n]
        return pltpu.make_async_copy(src.at[:, pl.ds(pl.multiple_of(j * FC, FC), FC)], dst.at[s], wsem.at[2 * n + s])

    def x_tiles(q):
        return [f'x{n}' for n in range(4 * q, 4 * q + 4)]

    def to_columns(row):
        return jnp.broadcast_to(row, (T, T)).T

    def silu_c():
        c = CV[...].astype(f32)
        s = _cat([c / (1.0 + jnp.exp(-c)), jnp.zeros((1, 5 * T - D), f32)], 1)
        for k in range(5):
            SB[_rows(k, T), :] = to_columns(s[:, _rows(k, T)])

    def mod(lo, hi):
        def gen():
            for j0 in range(lo, hi, 3):
                acc = [None] * 3
                for t in range(D // 16):
                    s = SB[_rows(t), :]
                    for u in range(3):
                        v = mul(_cast(WM[_rows(t), _rows(j0 + u, T)], f32), s)
                        acc[u] = v if t == 0 else add(acc[u], v)
                    yield 18
                for u in range(3):
                    row = jnp.sum(acc[u], axis=0, keepdims=True)
                    n = (j0 + u) * T + lax.broadcasted_iota(jnp.int32, (1, T), 1)
                    is_scale = ((n >= CA) & (n < CA + D)) | ((n >= CB) & (n < CB + D))
                    row = jnp.where(is_scale, 1.0 + row, row)
                    row = row * jnp.where(n >= GB2, 0.5 / GS, jnp.where(n >= SB2, GS, 1.0))
                    ROW[j0 + u] = jnp.broadcast_to(row, (8, T))
                    traced.append(j0 + u)
        return gen(), (hi - lo) * 6 * (D // 16)

    def biases():
        B1[...] = GS * B1V[...].astype(f32).reshape(1, F)
        b = 2.0 * GS * _cat([B2V[...].astype(f32).reshape(1, D), jnp.zeros((1, 5 * T - D), f32)], 1)
        for k in range(5):
            ROW[B2 // T + k] = jnp.broadcast_to(b[:, _rows(k, T)], (8, T))
            traced.append(B2 // T + k)

    def columns(lo, hi):
        def gen():
            for j in range(lo, hi):
                assert j in traced
                MOD[_rows(j, T), :] = _cat([ROW[j]] * (T // 8)).T
                yield 30
        return gen(), 30 * (hi - lo)

    def whole_tile(v):
        return v if v.shape[1] == T else _cat([v, jnp.zeros_like(v)], 1)

    def head_rows(k, base, d):
        return _cat(TURN[k % 4][pl.ds(k // 4 * 14 * T + base + d + e, 8, stride=DH), :] for e in range(2))

    def wqkv_transpose(lo, hi):
        def gen():
            for j in range(lo, hi):
                for k, halves in enumerate(DEPTH_TILES):
                    v = _cat(WQ[r:r + 64, j * T:min((j + 1) * T, 3 * D)] for r in halves).astype(f32)
                    TURN[k % 4][_rows(k // 4 * 14 + j, T), :] = whole_tile(v).T
                    yield 32
        return gen(), (hi - lo) * 6 * 32

    def wqkv_expand(m, g):
        def gen():
            for d in range(0, DH, 2):
                w = _once(lambda i, k: head_rows(k, m * D + (2 * g + i) * DB, d))
                for n in range(18):
                    WP[2 * m + g, n, _rows(d // 2), :] = _cast(_left_operand(n, w), bf16)
                    yield 4
            traced.append((m, g))
        return gen(), 9 * 18 * 4

    def wo_stage():
        def gen():
            for j in range(5):
                for k in range(D // 64):
                    v = WO[_rows(k, 64), j * T:min((j + 1) * T, D)].astype(f32)
                    TURN[j % 4][_rows(j // 4 * 28 + k, 64), :] = whole_tile(v)
                    yield 8
        return gen(), 45 * 8

    def wo_transpose():
        def gen():
            for j in range(5):
                parts = [head_rows(j, g * DB, d) for g in range(4) for d in range(0, DH, 2)]
                a, b, c = parts[24:28], parts[28:32], parts[32:36]
                parts = parts[:24] + a + c + a + b + b + c
                for k in range(6):
                    v = _cat(parts[8 * k:8 * k + 8]).T.astype(bf16)
                    for r in range(j * T, min((j + 1) * T, D), 16):
                        WOP[r // DB, k, _rows(0, 16, r % DB), :] = v[_rows(0, 16, r % T)]
                    yield 40
        return gen(), 30 * 40

    lane = lax.broadcasted_iota(jnp.int32, (8, T), 1)
    quarter = lane // 32

    def by_quarter(v):
        even, low = quarter % 2 == 0, quarter < 2
        half = [lax.select(even, v[-i % 4], v[(1 - i) % 4]) for i in range(4)]
        return [lax.select(low, half[i], half[(i + 2) % 4]) for i in range(4)]

    def deal_within(q):
        def gen():
            for s in range(4):
                src = (lane % 32 // 2) * 8 + ((quarter + 4 - s) % 4) * 2 + lane % 2
                for t in range(D // 16):
                    TT[q, s, _rows(t, 8), :] = jnp.take_along_axis(XB.bitcast(u32)[4 * q + s, _rows(t, 8), :], src, axis=1)
                    yield 2
        return gen(), 8 * 36

    def deal_across(q):
        def gen():
            for t in range(D // 16):
                for i, u in enumerate(by_quarter([TT[q, s, _rows(t, 8), :] for s in range(4)])):
                    MIX[4 * q + i, _rows(t, 8), :] = pltpu.roll(u, T - 32 * i, 1) if i else u
                yield 12
        return gen(), 12 * 36

    def collect_across(q, t):
        v = [XB.bitcast(u32)[4 * q + i, _rows(t, 8), :] for i in range(4)]
        for s, u in enumerate(by_quarter([pltpu.roll(v[i], 32 * i, 1) if i else v[0] for i in range(4)])):
            TT[q, s, _rows(t, 8), :] = u

    def collect_within(q, lo=0, hi=D // 16):
        def gen():
            for s in range(4):
                src = ((lane % 8 // 2 + s) % 4) * 32 + (lane // 8) * 2 + lane % 2
                for t in range(lo, hi):
                    u = jnp.take_along_axis(TT[q, s, _rows(t, 8), :], src, axis=1)
                    OUT[_rows(t), _rows(4 * q + s, T)] = pltpu.bitcast(u, bf16)
                    yield 2
        return gen(), (hi - lo) * 8

    def dealt(tile, t):
        return _cast(pltpu.bitcast(MIX[tile, _rows(t, 8), :], bf16), f32)

    def moments(tile, load, cost):
        for t in range(D // 16):
            v = load(t)
            if t == 0:
                pivot = jnp.broadcast_to(jnp.sum(v, axis=0, keepdims=True) * (1.0 / 16), (16, T))
            dv = sub(v, pivot)
            s1, s2 = (dv, mul(dv, dv)) if t == 0 else (add(s1, dv), add(s2, mul(dv, dv)))
            yield cost
        m1 = jnp.sum(s1, axis=0, keepdims=True) * (1.0 / D)
        m2 = jnp.sum(s2, axis=0, keepdims=True) * (1.0 / D)
        STAT[tile, 0] = pivot[:8] + m1
        STAT[tile, 1] = jnp.broadcast_to(lax.rsqrt(jnp.maximum(m2 - m1 * m1, 0.0) + EPS), (8, T))

    def normaliser():
        stat = _once(lambda tile, k: _cat([STAT[tile, k]] * 2))
        return lambda v, tile: mul(sub(v, stat(tile, 0)), stat(tile, 1))

    def modulate(v, t, scale, shift):
        return add(mul(v, MOD[_rows(t, 16, scale), :]), MOD[_rows(t, 16, shift), :])

    def ln1_moments(q):
        def gen():
            for tile in range(4 * q, 4 * q + 4):
                yield from moments(tile, lambda t: dealt(tile, t), 10)
        return gen(), 4 * 36 * 10

    def ln1_scale(q):
        normalise = normaliser()
        for i in range(4):
            for t in range(D // 16):
                X1[q][i, _rows(t), :] = normalise(dealt(4 * q + i, t), 4 * q + i)

    def ln1_apply(q, scaled=False):
        def gen():
            normalise = normaliser()

            def put(i, n, t, v):
                H1[2 * q + i, n, _rows(t), :] = _cast(v, bf16)

            def load(i, n):
                v = X1[q][i, _rows(n), :] if scaled else normalise(dealt(4 * q + i, n), 4 * q + i)
                return modulate(v, n, CA, SA)

            for t in range(8):
                first = []
                for i in range(2):
                    h = _once(lambda n, j: load(2 * i + j, n))
                    first.append([_right_operand(n, t, h) for n in range(2 if t < 4 else 1)])
                    for n in range(2, 14):
                        put(i, n, t, _right_operand(n, t, h))
                        yield 12
                    for n in range(14, 17 if t >= 4 else 0):
                        for u in (t - 4, t):
                            put(i, n, u, _right_operand(n, u, h))
                if t < 4:
                    put(0, 0, t, first[0][0])
                    put(1, 1, 4 + t, first[1][0])
                    put(0, 1, t, first[0][1])
                    put(1, 1, t, sub(first[1][1], first[0][1]))
                else:
                    put(0, 1, t, first[1][0])
                    put(0, 0, t, sub(first[0][0], first[1][0]))
        return gen(), 2 * 8 * 12 * 12

    def ln2_moments(q):
        def gen():
            for i in range(4):
                def residual(t):
                    v = add(dealt(4 * q + i, t), mul(MOD[_rows(t, 16, GA), :], X1[q][i, _rows(t), :]))
                    X1[q][i, _rows(t), :] = v
                    return v
                yield from moments(4 * q + i, residual, 14)
            traced.append(('ln2', q))
        return gen(), 4 * 36 * 14

    def ln2_apply(q):
        def gen():
            assert ('ln2', q) in traced
            normalise = normaliser()
            for t in range(9):
                blk = {}
                for k in range(4):
                    for i in range(4):
                        blk[k, i] = modulate(normalise(X1[q][i, _rows(4 * t + k), :], 4 * q + i), 4 * t + k, CB, SB2)
                        if t == 8:
                            HB[q][NP + i, _rows(k), :] = _cast(blk[k, i], bf16)
                        yield 8

                def emit(p, v):
                    HB[q][p, _rows(t), :] = v
                yield from _expand(B_TERMS, blk, emit)
        return gen(), 9 * (128 + EXPAND_COST)

    def project(q, m, pairs=(0, 1)):
        def gen():
            for g in pairs:
                assert (m, g) in traced
                both = _dot(_ld(WP, 2 * m + g, 17), _ld(H1, 2 * q, 1))
                yield DB
                for i in range(2):
                    def part(tiles, acc=None):
                        for n in tiles:
                            v = _dot(_ld(WP, 2 * m + g, n), _ld(H1, 2 * q + i, n))
                            acc = v if acc is None else add(acc, v)
                            yield DB
                        return [acc]
                    out = yield from _sum_products(lambda p: part((2 * p, 2 * p + 1)) if p else part((i,), both),
                                                   lambda p: part((14 + p,)))
                    for n, (v,) in enumerate(out):
                        QKV[q][qkv_rows(2 * i + n % 2, m * D + (2 * g + n // 2) * DB, DB), :] = v
        return gen(), len(pairs) * 33 * DB

    def first_value():
        def gen():
            for row in range(0, D, 8):
                V0[row:row + 8, :] = jnp.take_along_axis(QKV[0][qkv_rows(0, 2 * D + row), :], lane * 0, axis=1)
                yield 2
        return gen(), D // 4

    def attend(q):
        logit, prob = {}, {}
        from_lane = _once(lambda n: lane >= n)

        def tile(row, j):
            back = -2 * (j // 4)
            v = QKV[q][qkv_rows(j % 4, row), :]
            if back and q:
                v = lax.select(from_lane(T - back), QKV[q - 1][qkv_rows(j % 4, row), :], v)
            if back:
                v = pltpu.roll(v, back, 1)
            if back and not q and row >= 2 * D:
                v = lax.select(from_lane(back), v, V0[_rows(0, 8, row - 2 * D), :])
            return v

        def users(j):
            return [i for i in range(4) if 0 <= i - j < WIN]

        def score(g):
            def gen():
                for js in ((3, 0, -1, -4, -7), (2, 1, -2, -3, -5, -6)):
                    for d in range(DH):
                        row = g * DB + d * 8
                        query = _once(lambda i: tile(row, i))
                        for j in js:
                            k = tile(D + row, j)
                            for i in users(j):
                                u = mul(query(i), k)
                                logit[i, j] = u if d == 0 else add(logit[i, j], u)
                            yield 2 * len(users(j))
            return gen(), DH * 64

        def softmax(g):
            def gen():
                for i in range(4):
                    js = [i - w for w in range(WIN)]
                    z = [logit[i, j] * (SCALE * LOG2E) for j in js]
                    if q == 0:
                        z = [jnp.where(from_lane(-2 * (j // 4)), u, -1e9 * LOG2E) if j < 0 else u
                             for j, u in zip(js, z)]
                    top = z[0]
                    for u in z[1:]:
                        top = lax.max(top, u)
                    e = [lax.exp2(sub(u, top)) for u in z]
                    inv = 1.0 / (((e[0] + e[1]) + (e[2] + e[3])) + ((e[4] + e[5]) + (e[6] + e[7])))
                    for j, u in zip(js, e):
                        prob[i, j] = mul(u, inv)
                    yield 50
            return gen(), 200

        def mix(g):
            def gen():
                for row in range(g * DB, (g + 1) * DB, 16):
                    o = {}
                    for j in (3, -1, -2, 2, -3, -4, 1, -5, -6, 0, -7):
                        v = [tile(2 * D + row + h, j) for h in (0, 8)]
                        for i in users(j):
                            for h in range(2):
                                u = mul(prob[i, j], v[h])
                                o[i, h] = add(o[i, h], u) if (i, h) in o else u
                        yield 4 * len(users(j))
                    for n in range(2):
                        u, v = (_cat([o[i, 0], o[i, 1]]) for i in (2 * n, 2 * n + 1))
                        slab, r = divmod(row, 64)
                        if slab < 7:
                            put = ((row, u), (4 * T + row, v))
                        elif slab == 7:
                            put = ((8 * T + r, u), (4 * T + row, sub(v, u)))
                        else:
                            put = ((7 * 64 + r, sub(u, v)), (8 * T + 64 + r, v))
                        for r, w in put:
                            OB[2 * q + n, r:r + 16, :] = _cast(w, bf16)
            return gen(), DH * 64

        return _chain([f(g) for g in range(4) for f in (score, softmax, mix)])

    def project_out(q):
        def gen():
            for g in range(4):
                for n in range(2):
                    both = _dot(_ld(WOP, g, 5), _ld(OB, 2 * q + n, _rows(8, T // 2)))
                    yield DB
                    for i in range(2):
                        acc = both
                        for k in range(4):
                            w = _ld(WOP, g, k if k < 3 else 3 + i)
                            acc = add(acc, _dot(w, _ld(OB, 2 * q + n, _rows(4 * i + k, T // 2))))
                            if k == 3:
                                X1[q][2 * n + i, _rows(g, DB), :] = acc
                            yield DB
        return gen(), 72 * DB

    def slabs(j, among, load):
        if isinstance(j, int):
            return [load(8 if j == t else t) for t in range(8)]
        return [jnp.where(j == t, load(8), load(t)) if t in among else load(t) for t in range(8)]

    def is_chunk(j, n):
        return isinstance(j, int) and j == n

    def w1_transpose(j, s):
        def gen():
            for i in range(4):
                for k in range(4):
                    def load(n):
                        at = _rows(4 * n + k), _rows(i, T)
                        if is_chunk(j, SHARED):
                            return _cast(WS[at], f32)
                        v = _cast(W1R[(s, *at)], f32)
                        return v if n == 8 else sub(v, _cast(WS[at], f32))
                    WT[s, i, k, 0:T, :] = _cat(slabs(j, range(6 - s, 8, 2), load)).T
                    yield 64
        return gen(), 16 * 64

    def w1_last_slab():
        for i in range(4):
            v = W1R[(NC - 1) % 2, 4 * T:D, _rows(i, T)]
            WL[i] = _cat([v, jnp.zeros_like(v)]).T

    def w1_expand(j, s, lo=0, hi=8):
        def gen():
            for t in range(lo, hi):
                def emit(p, v):
                    W1[s][p, _rows(t), :] = v
                yield from _expand(A_TERMS, {(i, k): WT[s, i, k, _rows(t), :] for i in range(4) for k in range(4)}, emit)
                if t % 2 and not is_chunk(j, SHARED):
                    BC[s, t // 2] = to_columns(B1[:, pl.ds(pl.multiple_of(j * FC + t // 2 * T, T), T)])
            traced.append(('w1', s))
        return gen(), (hi - lo) * EXPAND_COST

    def w2_expand(s, lo, hi):
        def gen():
            for t in range(lo, hi):
                blk = {}
                for d in range(4):
                    for k in range(4):
                        blk[d, k] = _cast(W2R[s, _rows(4 * t + d), _rows(k, T)], f32)
                        yield 2

                def emit(p, v):
                    W2[s][p, _rows(t), :] = v
                yield from _expand(A_TERMS, blk, emit)
        return gen(), (hi - lo) * (32 + EXPAND_COST)

    def up(j, s, q):
        extra = 16 if is_chunk(j, NC - 1) else 0

        def gen():
            assert ('w1', s) in traced
            words = HB[q].bitcast(u32)
            for p in range(NP):
                h = _cat(slabs(j, range(4 - s, 7, 2), _once(lambda n: words[p, _rows(n, 8), :])))
                v = _dot(_ld(W1[s], p), pltpu.bitcast(h, bf16))
                if p in ROW_PRODUCTS and not is_chunk(j, SHARED):
                    v = add(v, BC[s, ROW_PRODUCTS.index(p)])
                M1[s][q][product_rows(p), :] = v
                yield T
            for n in range(extra):
                M1[s][q][product_rows(NP + n), :] = _dot(_ld(WL, n // 4), _ld(HB[q], NP + n % 4, slice(0, T // 2)))
                yield T
        return gen(), (NP + extra) * T

    def keep_shared(q):
        def gen():
            for r in range(0, T, 8):
                z = yield from _contract(lambda p: M1[1][q][product_rows(p, r, 8), :])
                for (c, i), v in z.items():
                    Z[q][product_rows(4 * c + i, r, 8), :] = v
                    yield 1
        return gen(), 16 * (2 * NP + 16)

    def activate(j, s, q, lo=0, hi=8):
        rest, at = (M1[s][q], NP) if is_chunk(j, NC - 1) else (Z[q], 0)
        plain = is_chunk(j, NC - 1) and q == NQ - 1

        def gen():
            for t in range(lo, hi):
                halves = []
                for r in (16 * t, 16 * t + 8):
                    pre = yield from _contract(lambda p: M1[s][q][product_rows(p, r, 8), :])
                    for (c, i), u in pre.items():
                        u = add(u, rest[product_rows(at + 4 * c + i, r, 8), :])
                        pre[c, i] = add(mul(u, lax.tanh(mul(u, add(mul(u, u), GK)))), u)
                        yield GELU_COST
                    halves.append(pre)
                blk = {k: _cat([halves[0][k], halves[1][k]]) for k in halves[0]}

                def emit(p, v):
                    GB[s][q][p, _rows(t), :] = v
                if plain:
                    for (c, i), v in blk.items():
                        emit(4 * c + i, _cast(v, bf16))
                else:
                    yield from _expand(B_TERMS, blk, emit)
        return gen(), (hi - lo) * (4 * NP + 32 * GELU_COST + (0 if plain else EXPAND_COST))

    def down(s, q, first=False):
        def gen():
            for p in range(NP):
                v = _dot(_ld(W2[s], p), _ld(GB[s][q], p))
                if not first:
                    v = add(v, ACC[q][p])
                elif p in ROW_PRODUCTS:
                    v = add(v, _cat(MOD[_rows(n, 16, B2), :] for n in range(ROW_PRODUCTS.index(p), D // 16, 4)))
                ACC[q][p] = v
                yield DB
        return gen(), NP * DB

    def finish(q, lo=0, hi=DB // 16):
        def gen():
            for t in range(lo, hi):
                halves = []
                for r in (_rows(2 * t, 8), _rows(2 * t + 1, 8)):
                    halves.append((yield from _contract(lambda p: ACC[q][p, r, :])))
                done = q < NQ - 1 or 64 * t < LAST[2]
                for d in range(4):
                    r = _rows(4 * t + d)
                    gate = MOD[_rows(4 * t + d, 16, GB2), :]
                    for i in range(4):
                        y = add(X1[q][i, r, :], mul(gate, _cat([halves[0][d, i], halves[1][d, i]])))
                        if done:
                            XB[4 * q + i, r, :] = _cast(y, bf16)
                        else:
                            X1[q][i, r, :] = y
                        yield 5
                    if done:
                        collect_across(q, 4 * t + d)
                    yield 12
        return gen(), (hi - lo) * (4 * NP + 16 * 5 + 48)

    def down_last(d):
        q, s, (lo, hi) = NQ - 1, (NC - 1) % 2, LAST[d:d + 2]

        def gen():
            for i in range(4):
                for k in range(4):
                    v = _dot(W2R[s, lo:hi, _rows(k, T)], _ld(GB[s][q], 4 * k + i))
                    acc = v if k == 0 else add(acc, v)
                    yield hi - lo
                y = add(X1[q][i, lo:hi, :], mul(MOD[GB2 + lo:GB2 + hi, :], acc))
                if d < 2:
                    X1[q][i, lo:hi, :] = y
                else:
                    XB[4 * q + i, lo:hi, :] = _cast(y, bf16)
            traced.append(('last', d))
        return gen(), 16 * (hi - lo)

    def send_last(d):
        assert ('last', d) in traced
        for t in range(LAST[d] // 16, LAST[d + 1] // 16):
            collect_across(NQ - 1, t)
        _trace([collect_within(NQ - 1, LAST[d] // 16, LAST[d + 1] // 16)])
        start(f'out3{d}')

    start('c', *x_tiles(0), 'wk0', 'wm0', 'wm1', 'wm2', 'wk1')

    @pl.loop(0, 4)
    def _(n):
        flag[0] = n

    for q in range(NQ):
        HB[q][NP:, 64:T, :] = jnp.zeros((4, 64, T), bf16)

    def block(*lists):
        pl.when(flag[0] >= 0)(lambda: _trace(*lists))

    def ln1(q):
        return [ln1_moments(q), ln1_apply(q)]

    def activate_all(j, s, groups=range(NQ)):
        return [v for q in groups for v in _pieces(activate, j, s, q)]

    shared = [f'ws{n}' for n in range(8)]
    wait('c')
    silu_c()
    wait(*x_tiles(0))
    block([deal_within(0), deal_across(0)])
    wait('wk0')
    block([wqkv_transpose(4, 7), wqkv_expand(1, 0)], [ln1_moments(0)])
    block([_call(ln1_scale, 0)])
    wait('wm0', 'wm1')
    start('wq1', 'wq0')
    block([mod(0, 6), columns(0, 6)])
    wait('wm2')
    start(*x_tiles(1), 'wv')
    block([mod(6, 9), columns(6, 9), ln1_apply(0, True)])
    wait('wk1')
    block([project(0, 1, (0,))], [wqkv_transpose(7, 9), wqkv_expand(1, 1)])
    wait('wq1')
    block([project(0, 1, (1,))], [wqkv_transpose(2, 4), wqkv_expand(0, 1)])
    wait('wq0', *x_tiles(1))
    start(*x_tiles(2))
    block([project(0, 0, (1,))], [wqkv_transpose(0, 2), wqkv_expand(0, 0)], [deal_within(1)])
    wait('wv')
    start(*x_tiles(3))
    block([project(0, 0, (0,))], [wqkv_transpose(9, 14), wqkv_expand(2, 0), deal_across(1)])
    wait(*x_tiles(2))
    start('wo', 'b1', 'b2')
    block([project(0, 2)], [wqkv_expand(2, 1)] + ln1(1), [deal_within(2), deal_across(2)])
    wait(*x_tiles(3), 'wo', 'b1', 'b2')
    block([project(1, 1)], ln1(2), [deal_within(3), first_value(), deal_across(3)], [wo_stage(), _call(biases)])
    block([project(1, 0), project(1, 2), project(2, 1)], [attend(0), wo_transpose()],
          [ln1_moments(3), _call(start, 'wm3', *shared), ln1_apply(3)])
    wait('wm3', *shared)
    chunk(0, 0, 0).start()
    block([project(2, 0), project(2, 2), project_out(0)], [attend(1), w1_transpose(SHARED, 1), columns(9, 24)],
          [mod(9, 24), _idle(900)])
    chunk(0, 0, 0).wait()
    chunk(0, 1, 1).start()
    block([project(3, 0), project(3, 1), project(3, 2), project_out(1)],
          [attend(2), w1_expand(SHARED, 1), ln2_apply(0)], [ln2_moments(0), w1_transpose(0, 0)])
    chunk(1, 0, 0).start()
    chunk(0, 2, 0).start()
    block([project_out(2), up(SHARED, 1, 0), up(0, 0, 0)], [w1_expand(0, 0), attend(3)], [ln2_moments(1)])
    chunk(1, 1, 1).start()
    block([project_out(3)], [ln2_apply(1), ln2_moments(2)], [columns(27, 32)])
    block([up(SHARED, 1, 1), up(0, 0, 1)], [ln2_moments(3), keep_shared(0), ln2_apply(2), ln2_apply(3)])
    chunk(0, 1, 1).wait()
    chunk(1, 0, 0).wait()
    block([up(SHARED, 1, 2), up(SHARED, 1, 3), up(0, 0, 2), up(0, 0, 3)],
          [keep_shared(1)] + _in_turns(activate_all(0, 0, (0, 1)), _pieces(w2_expand, 0, hi=9)), [w1_transpose(1, 1)])
    chunk(0, 3, 1).start()
    chunk(1, 2, 0).start()
    chunk(0, 2, 0).wait()
    block([down(0, 0, True), down(0, 1, True)], [keep_shared(2), w1_expand(1, 1), keep_shared(3)], [w1_transpose(2, 0)])
    chunk(0, 4, 0).start()
    chunk(0, 3, 1).wait()
    chunk(1, 1, 1).wait()
    block([up(1, 1, q) for q in range(NQ)],
          _in_turns(activate_all(0, 0, (2, 3)), _pieces(w1_expand, 2, 0) + _pieces(w2_expand, 1, hi=5)), [w1_transpose(3, 1)])
    chunk(0, 5, 1).start()
    chunk(0, 4, 0).wait()
    start('wm4')
    block([_merge([[up(2, 0, q) for q in range(NQ)], [down(0, 2, True), down(0, 3, True)]], 3)],
          _in_turns(activate_all(1, 1), _pieces(w2_expand, 1, lo=5, hi=9) + _pieces(w1_expand, 3, 1)), [w1_transpose(4, 0)])

    def step(j, s, turn):
        chunk(1, j, s).wait()
        chunk(1, j + 1, 1 - s).start()
        block([_merge([[up(j + 1, 1 - s, q) for q in range(NQ)], [down(1 - s, q) for q in range(NQ)]], RUN)],
              _in_turns(activate_all(j, s), _pieces(w2_expand, s, hi=9) + _pieces(w1_expand, j + 2, s)), [turn])

    @pl.loop(1, 3)
    def _(n):
        j = 2 * n
        chunk(0, j + 3, 1).wait()
        chunk(0, j + 4, 0).start()
        step(j, 0, w1_transpose(j + 3, 1))
        chunk(0, j + 4, 0).wait()
        pl.when(j + 5 < NC)(lambda: chunk(0, j + 5, 1).start())

        @pl.when(j + 4 == NC - 1)
        def _():
            WS[...] = jnp.zeros(WS.shape, bf16)
        step(j + 1, 1, w1_transpose(j + 4, 0))

    step(6, 0, _call(w1_last_slab))
    chunk(1, 7, 1).wait()
    wait('wm4')
    chunk(1, 8, 0).start()
    block([_merge([[up(8, 0, 0), up(8, 0, 1)], [down(0, q) for q in range(NQ)]], 3)],
          _in_turns(activate_all(7, 1)[:-3], _pieces(w2_expand, 1, hi=9)), [mod(24, 27)])
    chunk(1, 8, 0).wait()
    block([_merge([[up(8, 0, 2), up(8, 0, 3)], [down(1, 0)]], 4)],
          _in_turns(activate_all(8, 0, (0, 1)), _pieces(w2_expand, 0, hi=9)))
    block([down(0, 0), down(1, 1)], [activate(8, 0, 2), activate(7, 1, 3, 5, 8)], [columns(24, 27)])
    block([down(0, 1), down(1, 2)], _in_turns(activate_all(8, 0, (3,)), _pieces(finish, 0, hi=9)))
    block([down(0, 2)], [finish(1)], [collect_within(0)])
    start('out0')
    block([down(1, 3)], [finish(2)], [collect_within(1)])
    start('out1')
    block([down_last(0), down_last(1)], [finish(3, 4, 9)], [collect_within(2)])
    start('out2')
    block([down_last(2), down_last(3)],
          [finish(3, 0, 4), collect_within(3, 0, 16), _call(start, 'out31'), _call(send_last, 2), _idle(400)])
    block([_call(send_last, 3)])
    wait(*[k for k in copies if k.startswith('out')])


@jax.jit
def pallas_adaLN_cond__sliding_local_dilated__dense_activation_gelu__prompt_kernel(
    A_x: jax.Array,
    A_wqkv: jax.Array,
    A_wo: jax.Array,
    B_x: jax.Array,
    B_w1: jax.Array,
    B_b1: jax.Array,
    B_w2: jax.Array,
    B_b2: jax.Array,
    c: jax.Array,
    w_mod: jax.Array,
):
    del B_x
    assert A_x.shape == (1, S, D) and B_w1.shape == (D, F)
    vmem = pltpu.VMEM
    scratch = [
        vmem((4 * NQ, D, T), bf16),
        vmem((D, 6 * D), bf16),
        vmem((D, 3 * D), bf16),
        vmem((D, D), bf16),
        vmem((2, D, FC), bf16),
        vmem((2, D, FC), bf16),
        vmem((4 * T, FC), bf16),
        vmem((F,), bf16), vmem((D,), bf16), vmem((1, D), bf16),
        vmem((1, F), f32),
        vmem((5 * T, T), f32),
        vmem((D, T), f32),
        vmem((32, 8, T), f32),
        vmem((32 * T, T), f32),
        vmem((6, 18, DB, T), bf16),
        vmem((4, 6, DB, T), bf16),
        vmem((4 * NQ, D // 2, T), u32),
        vmem((2 * NQ, 17, T, T), bf16),
        vmem((4 * NQ, 2, 8, T), f32),
        vmem((NQ, 4, D // 2, T), u32),
        vmem((2 * NQ, 9 * T, T), bf16),
        [vmem((4, D, T), f32)] * NQ,
        [vmem((NP + 4, DB, T), bf16)] * NQ,
        vmem((4, T, T), bf16),
        vmem((2, 4, 4, T + 8, T), f32),
        vmem((2, 4, T, T), f32),
        [vmem((NP, T, T), bf16)] * 2,
        [vmem((NP, DB, T), bf16)] * 2,
        [[vmem(((NP + 16) * (T + 8), T), f32)] * NQ, [vmem((12 * D, T), f32)] * NQ],
        [vmem((16 * (T + 8), T), f32)] * NQ,
        [[vmem((NP, T, T), bf16)] * NQ] * 2,
        [vmem((NP, DB, T), f32)] * NQ,
        pltpu.SMEM((1,), jnp.int32),
        pltpu.SemaphoreType.DMA((44,)),
        pltpu.SemaphoreType.DMA((4,)),
    ]
    out = pl.pallas_call(
        _kernel,
        out_shape=jax.ShapeDtypeStruct((D, S), A_x.dtype),
        in_specs=[pl.BlockSpec(memory_space=pl.ANY)] * 9,
        out_specs=pl.BlockSpec(memory_space=pl.ANY),
        scratch_shapes=scratch,
        compiler_params=pltpu.CompilerParams(
            vmem_limit_bytes=124 * 2**20,
            flags={'XLA_TPU_EVENLY_DISTRIBUTE_CRITICAL_NODES': True}),
        name='adaln_block',
    )(A_x[0].T, A_wqkv, A_wo, B_w1, B_b1, B_w2.T, B_b2, c, w_mod)
    return out.T[None]
```

```python
import jax
import jax.numpy as jnp
import numpy as np
from jax import lax
from jax.experimental import pallas as pl
from jax.experimental.pallas import tpu as pltpu

f32, bf16, u32 = jnp.float32, jnp.bfloat16, jnp.uint32
add, sub, mul = lax.add, lax.sub, lax.mul

S, D, F = 2048, 576, 4608
DH, WIN = 18, 8
T = 128
NQ = 4
DB = D // 4
FC = 4 * T
NC = F // FC
NP = 49
SHARED = -1
LAST = (0, 128, 256, 416, 576)
EPS = 1e-5
LOG2E = float(np.log2(np.e))
SCALE = float(DH ** -0.5)
GS = float(np.cbrt(np.sqrt(2.0 / np.pi) * 0.044715))
GK = np.float32(np.sqrt(2.0 / np.pi) / GS)

A_TERMS = (((1, 0, 0), (1, 1, 1)), ((1, 0, 1), (-1, 1, 1)), ((1, 0, 0), (1, 0, 1)), ((1, 1, 0), (-1, 0, 0)),
           ((1, 1, 0), (1, 1, 1)), ((1, 1, 1),), ((1, 0, 0),))
B_TERMS = (((1, 0, 0), (-1, 1, 1)), ((1, 1, 0), (-1, 1, 1)), ((1, 1, 1),), ((1, 0, 1), (-1, 0, 0)),
           ((1, 0, 0),), ((1, 1, 0), (-1, 0, 0)), ((1, 0, 1), (-1, 1, 1)))
ROW_PRODUCTS = tuple(7 * a + b for a in (2, 4) for b in (2, 4))
A_SLABS = (None, (0, 0), (2, 2), (0, 1), (1, 3), (1, 0), (2, 1),
           ((0, 0), (2, 2)), ((0, 1), (1, 3)), ((1, 0), (2, 1)))
B_SLABS = (None, (0, 0), (2, 0), (0, 1), (1, 1), (1, 2), (2, 3),
           ((0, 1), (2, 3)), ((0, 0), (1, 2)), ((1, 1), (2, 0)))
SLAB_ROW = (320, 448, 512)
DEPTH_TILES = ((0, 64), (128, 192), (256, 320), (384, 448), (320, 512), (448, 512))

STORE_COST = 3
GELU_COST = 7
RUN = 7
EXPAND_COST = 2 * 55 + STORE_COST * NP


def _cast(v, dtype):
    return lax.convert_element_type(v, dtype)


def _cat(vals, axis=0):
    return lax.concatenate(list(vals), axis)


def _dot(a, b):
    return lax.dot_general(a, b, (((1,), (0,)), ((), ())), preferred_element_type=f32)


def _ld(ref, *idx):
    return pltpu.bitcast(ref.bitcast(u32)[idx], bf16)


def _rows(t, n=16, at=0):
    return slice(at + t * n, at + (t + 1) * n)


def _once(fn):
    kept = {}

    def get(*key):
        if key not in kept:
            kept[key] = fn(*key)
        return kept[key]
    return get


def _combine(term, blk):
    v = blk(*term[0][1:])
    for sign, r, c in term[1:]:
        v = (add if sign > 0 else sub)(v, blk(r, c))
    return v


def _expand(terms, blk, emit):
    for p, outer in enumerate(terms):
        part = {}
        for r in range(2):
            for c in range(2):
                part[r, c] = _combine(outer, lambda i, j: blk[2 * i + r, 2 * j + c])
                yield 2 * (len(outer) - 1)
        for n, inner in enumerate(terms):
            emit(7 * p + n, _cast(_combine(inner, lambda r, c: part[r, c]), bf16))
            yield 2 * (len(inner) - 1) + STORE_COST


def _sum_products(m, extra=None):
    def plus(a, b):
        return [add(u, v) for u, v in zip(a, b)]

    c00, both = (yield from m(1)), (yield from m(2))
    c00, c01 = plus(c00, both), (plus((yield from extra(0)), both) if extra else both)
    c11, both = (yield from m(3)), (yield from m(4))
    c11, c10 = plus(c11, both), (plus((yield from extra(1)), both) if extra else both)
    diag = yield from m(0)
    c00, c11 = plus(c00, diag), [sub(u, v) for u, v in zip(c11, diag)]
    both = (yield from extra(2)) if extra else None
    col = yield from m(5)
    col = plus(col, both) if extra else col
    c00, c10 = plus(c00, col), plus(c10, col)
    col = yield from m(6)
    col = plus(col, both) if extra else col
    return [c00, plus(c01, col), c10, plus(c11, col)]


def _contract(get):
    def inner(p):
        def leaf(n):
            yield 2
            return [get(7 * p + n)]
        return [v[0] for v in (yield from _sum_products(leaf))]

    out = yield from _sum_products(inner)
    return {(2 * (a // 2) + b // 2, 2 * (a % 2) + b % 2): out[a][b] for a in range(4) for b in range(4)}


def _slab(op, blk):
    return blk(op) if op < 2 else sub(blk(op - 2), blk(3 - op))


def _left_operand(n, w):
    def slab(use, tiles):
        return _slab(use[1], lambda i: w(i, tiles[use[0]]))

    p, e = divmod(n, 2) if n < 14 else (n - 7, 0) if n < 17 else (0, 2)
    if p >= 7:
        low, high = slab(A_SLABS[p][0], (4, 5)), slab(A_SLABS[p][1], (2, 3, 4))
    elif e == 0:
        return _combine(A_TERMS[p], w)
    else:
        low = _combine(A_TERMS[p], lambda i, k: w(i, 2 + k))
        high = slab(A_SLABS[p], (2, 3, 4)) if p else _combine(A_TERMS[p], w)
        if n == 1:
            high = pltpu.roll(high, T // 2, 1)
    return lax.select(lax.broadcasted_iota(jnp.int32, low.shape, 1) < T // 2, low, high)


def _right_operand(n, t, h):
    def slab(use):
        return _slab(use[1], lambda j: h(SLAB_ROW[use[0]] // 16 + t % 4, j))

    p, e = divmod(n, 2)
    if n >= 14:
        return slab(B_SLABS[n - 7][t // 4])
    if e == 0 or t < 4:
        return _combine(B_TERMS[p], lambda k, j: h(16 * e + 8 * k + t, j))
    return slab(B_SLABS[p])


def _chain(streams):
    def gen():
        for g, _ in streams:
            yield from g
    return gen(), sum(c for _, c in streams)


def _merge(lists, run=1):
    def gen():
        live = [[*_chain(streams), 0.0] for streams in lists]
        while live:
            s = min(live, key=lambda z: z[2] / z[1])
            for _ in range(run):
                cost = next(s[0], None)
                if cost is None:
                    live.remove(s)
                    break
                s[2] += cost
                yield cost
    return gen(), sum(c for streams in lists for _, c in streams)


def _trace(*lists):
    for _ in _merge(lists)[0]:
        pass


def _in_turns(*lists):
    keyed = [((n + 0.5) / len(streams), k, v) for k, streams in enumerate(lists) for n, v in enumerate(streams)]
    return [v for _, _, v in sorted(keyed, key=lambda z: z[:2])]


def _pieces(fn, *args, lo=0, hi=8):
    return [fn(*args, t, t + 1) for t in range(lo, hi)]


def _call(fn, *args):
    def gen():
        fn(*args)
        yield 1
    return gen(), 1


def _idle(cost):
    return iter([cost]), cost


def _kernel(x_hbm, wqkv_hbm, wo_hbm, w1_hbm, b1_hbm, w2_hbm, b2_hbm, c_hbm, wm_hbm, o_hbm,
            XB, WM, WQ, WO, W1R, W2R, WS, B1V, B2V, CV, B1, SB, V0, ROW, MOD, WP, WOP, MIX, H1, STAT, TT,
            OB, X1, HB, WL, WT, BC, W1, W2, M1, Z, GB, ACC, flag, sem, wsem):
    SA, CA, GA, SB2, CB, GB2, B2 = (i * D for i in range(7))
    OUT = WM
    TURN, QKV = M1
    traced = []

    def qkv_rows(tile, row, n=8):
        return _rows(0, n, tile * 3 * D + row)

    def product_rows(p, row=0, n=T):
        return _rows(0, n, p * (T + 8) + row)

    def cols(src, dst, lo, hi):
        return src.at[:, lo:hi], dst.at[:, lo:hi]

    moves = dict(
        c=(c_hbm, CV), b1=(b1_hbm, B1V), b2=(b2_hbm, B2V), wo=(wo_hbm, WO),
        **{f'wm{n}': cols(wm_hbm, WM, lo * T, hi * T)
           for n, (lo, hi) in enumerate(((0, 3), (3, 6), (6, 9), (9, 24), (24, 27)))},
        **{k: cols(wqkv_hbm, WQ, lo * T, min(hi * T, 3 * D))
           for k, lo, hi in (('wq0', 0, 2), ('wq1', 2, 4), ('wk0', 4, 7), ('wk1', 7, 9), ('wv', 9, 14))},
        **{f'ws{n}': (w1_hbm.at[_rows(n, 64), _rows(n, FC)], WS.at[_rows(n, 64)]) for n in range(8)},
        **{f'x{n}': (x_hbm.at[:, _rows(n, T)], XB[n // 4].at[n % 4]) for n in range(4 * NQ)},
        **{f'out{q}': cols(OUT, o_hbm, q * FC, (q + 1) * FC) for q in range(NQ - 1)},
        **{f'out3{d}': tuple(r.at[LAST[d] if d > 1 else 0:LAST[d + 1], S - FC:S] for r in (OUT, o_hbm))
           for d in (1, 2, 3)})
    copies = {k: pltpu.make_async_copy(s, d, sem.at[i]) for i, (k, (s, d)) in enumerate(moves.items())}

    def start(*names):
        for k in names:
            copies[k].start()

    def wait(*names):
        for k in names:
            copies[k].wait()

    def chunk(n, j, s):
        src, dst = ((w1_hbm, W1R), (w2_hbm, W2R))[n]
        return pltpu.make_async_copy(src.at[:, pl.ds(pl.multiple_of(j * FC, FC), FC)], dst.at[s], wsem.at[2 * n + s])

    def x_tiles(q):
        return [f'x{n}' for n in range(4 * q, 4 * q + 4)]

    def to_columns(row):
        return jnp.broadcast_to(row, (T, T)).T

    def silu_c():
        c = CV[...].astype(f32)
        s = _cat([c / (1.0 + jnp.exp(-c)), jnp.zeros((1, 5 * T - D), f32)], 1)
        for k in range(5):
            SB[_rows(k, T), :] = to_columns(s[:, _rows(k, T)])

    def mod(lo, hi):
        def gen():
            for j0 in range(lo, hi, 3):
                acc = [None] * 3
                for t in range(D // 16):
                    s = SB[_rows(t), :]
                    for u in range(3):
                        v = mul(_cast(WM[_rows(t), _rows(j0 + u, T)], f32), s)
                        acc[u] = v if t == 0 else add(acc[u], v)
                    yield 18
                for u in range(3):
                    row = jnp.sum(acc[u], axis=0, keepdims=True)
                    n = (j0 + u) * T + lax.broadcasted_iota(jnp.int32, (1, T), 1)
                    is_scale = ((n >= CA) & (n < CA + D)) | ((n >= CB) & (n < CB + D))
                    row = jnp.where(is_scale, 1.0 + row, row)
                    row = row * jnp.where(n >= GB2, 0.5 / GS, jnp.where(n >= SB2, GS, 1.0))
                    ROW[j0 + u] = jnp.broadcast_to(row, (8, T))
                    traced.append(j0 + u)
        return gen(), (hi - lo) * 6 * (D // 16)

    def biases():
        B1[...] = GS * B1V[...].astype(f32).reshape(1, F)
        b = 2.0 * GS * _cat([B2V[...].astype(f32).reshape(1, D), jnp.zeros((1, 5 * T - D), f32)], 1)
        for k in range(5):
            ROW[B2 // T + k] = jnp.broadcast_to(b[:, _rows(k, T)], (8, T))
            traced.append(B2 // T + k)

    def columns(lo, hi):
        def gen():
            for j in range(lo, hi):
                assert j in traced
                MOD[_rows(j, T), :] = _cat([ROW[j]] * (T // 8)).T
                yield 30
        return gen(), 30 * (hi - lo)

    def whole_tile(v):
        return v if v.shape[1] == T else _cat([v, jnp.zeros_like(v)], 1)

    def head_rows(k, base, d):
        return _cat(TURN[k % 4][pl.ds(k // 4 * 14 * T + base + d + e, 8, stride=DH), :] for e in range(2))

    def wqkv_transpose(lo, hi):
        def gen():
            for j in range(lo, hi):
                for k, halves in enumerate(DEPTH_TILES):
                    v = _cat(WQ[r:r + 64, j * T:min((j + 1) * T, 3 * D)] for r in halves).astype(f32)
                    TURN[k % 4][_rows(k // 4 * 14 + j, T), :] = whole_tile(v).T
                    yield 32
        return gen(), (hi - lo) * 6 * 32

    def wqkv_expand(m, g):
        def gen():
            for d in range(0, DH, 2):
                w = _once(lambda i, k: head_rows(k, m * D + (2 * g + i) * DB, d))
                for n in range(18):
                    WP[2 * m + g, n, _rows(d // 2), :] = _cast(_left_operand(n, w), bf16)
                    yield 4
            traced.append((m, g))
        return gen(), 9 * 18 * 4

    def wo_stage():
        def gen():
            for j in range(5):
                for k in range(D // 64):
                    v = WO[_rows(k, 64), j * T:min((j + 1) * T, D)].astype(f32)
                    TURN[j % 4][_rows(j // 4 * 28 + k, 64), :] = whole_tile(v)
                    yield 8
        return gen(), 45 * 8

    def wo_transpose():
        def gen():
            for j in range(5):
                parts = [head_rows(j, g * DB, d) for g in range(4) for d in range(0, DH, 2)]
                a, b, c = parts[24:28], parts[28:32], parts[32:36]
                parts = parts[:24] + a + c + a + b + b + c
                for k in range(6):
                    v = _cat(parts[8 * k:8 * k + 8]).T.astype(bf16)
                    for r in range(j * T, min((j + 1) * T, D), 16):
                        WOP[r // DB, k, _rows(0, 16, r % DB), :] = v[_rows(0, 16, r % T)]
                    yield 40
        return gen(), 30 * 40

    lane = lax.broadcasted_iota(jnp.int32, (8, T), 1)
    quarter = lane // 32

    def by_quarter(v):
        even, low = quarter % 2 == 0, quarter < 2
        half = [lax.select(even, v[-i % 4], v[(1 - i) % 4]) for i in range(4)]
        return [lax.select(low, half[i], half[(i + 2) % 4]) for i in range(4)]

    def deal_within(q):
        def gen():
            for s in range(4):
                src = (lane % 32 // 2) * 8 + ((quarter + 4 - s) % 4) * 2 + lane % 2
                for t in range(D // 16):
                    TT[q, s, _rows(t, 8), :] = jnp.take_along_axis(XB[q].bitcast(u32)[s, _rows(t, 8), :], src, axis=1)
                    yield 2
        return gen(), 8 * 36

    def deal_across(q):
        def gen():
            for t in range(D // 16):
                for i, u in enumerate(by_quarter([TT[q, s, _rows(t, 8), :] for s in range(4)])):
                    MIX[4 * q + i, _rows(t, 8), :] = pltpu.roll(u, T - 32 * i, 1) if i else u
                yield 12
        return gen(), 12 * 36

    def collect_across(q, t):
        v = [XB[q].bitcast(u32)[i, _rows(t, 8), :] for i in range(4)]
        for s, u in enumerate(by_quarter([pltpu.roll(v[i], 32 * i, 1) if i else v[0] for i in range(4)])):
            TT[q, s, _rows(t, 8), :] = u

    def collect_within(q, lo=0, hi=D // 16):
        def gen():
            for s in range(4):
                src = ((lane % 8 // 2 + s) % 4) * 32 + (lane // 8) * 2 + lane % 2
                for t in range(lo, hi):
                    u = jnp.take_along_axis(TT[q, s, _rows(t, 8), :], src, axis=1)
                    OUT[_rows(t), _rows(4 * q + s, T)] = pltpu.bitcast(u, bf16)
                    yield 2
        return gen(), (hi - lo) * 8

    def dealt(tile, t):
        return _cast(pltpu.bitcast(MIX[tile, _rows(t, 8), :], bf16), f32)

    def moments(tile, load, cost):
        for t in range(D // 16):
            v = load(t)
            if t == 0:
                pivot = jnp.broadcast_to(jnp.sum(v, axis=0, keepdims=True) * (1.0 / 16), (16, T))
            dv = sub(v, pivot)
            s1, s2 = (dv, mul(dv, dv)) if t == 0 else (add(s1, dv), add(s2, mul(dv, dv)))
            yield cost
        m1 = jnp.sum(s1, axis=0, keepdims=True) * (1.0 / D)
        m2 = jnp.sum(s2, axis=0, keepdims=True) * (1.0 / D)
        STAT[tile, 0] = pivot[:8] + m1
        STAT[tile, 1] = jnp.broadcast_to(lax.rsqrt(jnp.maximum(m2 - m1 * m1, 0.0) + EPS), (8, T))

    def normaliser():
        stat = _once(lambda tile, k: _cat([STAT[tile, k]] * 2))
        return lambda v, tile: mul(sub(v, stat(tile, 0)), stat(tile, 1))

    def modulate(v, t, scale, shift):
        return add(mul(v, MOD[_rows(t, 16, scale), :]), MOD[_rows(t, 16, shift), :])

    def ln1_moments(q):
        def gen():
            for tile in range(4 * q, 4 * q + 4):
                yield from moments(tile, lambda t: dealt(tile, t), 10)
        return gen(), 4 * 36 * 10

    def ln1_scale(q):
        normalise = normaliser()
        for i in range(4):
            for t in range(D // 16):
                X1[q][i, _rows(t), :] = normalise(dealt(4 * q + i, t), 4 * q + i)

    def ln1_apply(q, scaled=False):
        def gen():
            normalise = normaliser()

            def put(i, n, t, v):
                H1[2 * q + i, n, _rows(t), :] = _cast(v, bf16)

            def load(i, n):
                v = X1[q][i, _rows(n), :] if scaled else normalise(dealt(4 * q + i, n), 4 * q + i)
                return modulate(v, n, CA, SA)

            for t in range(8):
                first = []
                for i in range(2):
                    h = _once(lambda n, j: load(2 * i + j, n))
                    first.append([_right_operand(n, t, h) for n in range(2 if t < 4 else 1)])
                    for n in range(2, 14):
                        put(i, n, t, _right_operand(n, t, h))
                        yield 12
                    for n in range(14, 17 if t >= 4 else 0):
                        for u in (t - 4, t):
                            put(i, n, u, _right_operand(n, u, h))
                if t < 4:
                    put(0, 0, t, first[0][0])
                    put(1, 1, 4 + t, first[1][0])
                    put(0, 1, t, first[0][1])
                    put(1, 1, t, sub(first[1][1], first[0][1]))
                else:
                    put(0, 1, t, first[1][0])
                    put(0, 0, t, sub(first[0][0], first[1][0]))
        return gen(), 2 * 8 * 12 * 12

    def ln2_moments(q):
        def gen():
            for i in range(4):
                def residual(t):
                    v = add(dealt(4 * q + i, t), mul(MOD[_rows(t, 16, GA), :], X1[q][i, _rows(t), :]))
                    X1[q][i, _rows(t), :] = v
                    return v
                yield from moments(4 * q + i, residual, 14)
            traced.append(('ln2', q))
        return gen(), 4 * 36 * 14

    def ln2_apply(q):
        def gen():
            assert ('ln2', q) in traced
            normalise = normaliser()
            for t in range(9):
                blk = {}
                for k in range(4):
                    for i in range(4):
                        blk[k, i] = modulate(normalise(X1[q][i, _rows(4 * t + k), :], 4 * q + i), 4 * t + k, CB, SB2)
                        if t == 8:
                            HB[q][NP + i, _rows(k), :] = _cast(blk[k, i], bf16)
                        yield 8

                def emit(p, v):
                    HB[q][p, _rows(t), :] = v
                yield from _expand(B_TERMS, blk, emit)
        return gen(), 9 * (128 + EXPAND_COST)

    def project(q, m, pairs=(0, 1)):
        def gen():
            for g in pairs:
                assert (m, g) in traced
                both = _dot(_ld(WP, 2 * m + g, 17), _ld(H1, 2 * q, 1))
                yield DB
                for i in range(2):
                    def part(tiles, acc=None):
                        for n in tiles:
                            v = _dot(_ld(WP, 2 * m + g, n), _ld(H1, 2 * q + i, n))
                            acc = v if acc is None else add(acc, v)
                            yield DB
                        return [acc]
                    out = yield from _sum_products(lambda p: part((2 * p, 2 * p + 1)) if p else part((i,), both),
                                                   lambda p: part((14 + p,)))
                    for n, (v,) in enumerate(out):
                        QKV[q][qkv_rows(2 * i + n % 2, m * D + (2 * g + n // 2) * DB, DB), :] = v
        return gen(), len(pairs) * 33 * DB

    def first_value():
        def gen():
            for row in range(0, D, 8):
                V0[row:row + 8, :] = jnp.take_along_axis(QKV[0][qkv_rows(0, 2 * D + row), :], lane * 0, axis=1)
                yield 2
        return gen(), D // 4

    def attend(q):
        logit, prob = {}, {}
        from_lane = _once(lambda n: lane >= n)

        def tile(row, j):
            back = -2 * (j // 4)
            v = QKV[q][qkv_rows(j % 4, row), :]
            if back and q:
                v = lax.select(from_lane(T - back), QKV[q - 1][qkv_rows(j % 4, row), :], v)
            if back:
                v = pltpu.roll(v, back, 1)
            if back and not q and row >= 2 * D:
                v = lax.select(from_lane(back), v, V0[_rows(0, 8, row - 2 * D), :])
            return v

        def users(j):
            return [i for i in range(4) if 0 <= i - j < WIN]

        def score(g):
            def gen():
                for js in ((3, 0, -1, -4, -7), (2, 1, -2, -3, -5, -6)):
                    for d in range(DH):
                        row = g * DB + d * 8
                        query = _once(lambda i: tile(row, i))
                        for j in js:
                            k = tile(D + row, j)
                            for i in users(j):
                                u = mul(query(i), k)
                                logit[i, j] = u if d == 0 else add(logit[i, j], u)
                            yield 2 * len(users(j))
            return gen(), DH * 64

        def softmax(g):
            def gen():
                for i in range(4):
                    js = [i - w for w in range(WIN)]
                    z = [logit[i, j] * (SCALE * LOG2E) for j in js]
                    if q == 0:
                        z = [jnp.where(from_lane(-2 * (j // 4)), u, -1e9 * LOG2E) if j < 0 else u
                             for j, u in zip(js, z)]
                    top = z[0]
                    for u in z[1:]:
                        top = lax.max(top, u)
                    e = [lax.exp2(sub(u, top)) for u in z]
                    inv = 1.0 / (((e[0] + e[1]) + (e[2] + e[3])) + ((e[4] + e[5]) + (e[6] + e[7])))
                    for j, u in zip(js, e):
                        prob[i, j] = mul(u, inv)
                    yield 50
            return gen(), 200

        def mix(g):
            def gen():
                for row in range(g * DB, (g + 1) * DB, 16):
                    o = {}
                    for j in (3, -1, -2, 2, -3, -4, 1, -5, -6, 0, -7):
                        v = [tile(2 * D + row + h, j) for h in (0, 8)]
                        for i in users(j):
                            for h in range(2):
                                u = mul(prob[i, j], v[h])
                                o[i, h] = add(o[i, h], u) if (i, h) in o else u
                        yield 4 * len(users(j))
                    for n in range(2):
                        u, v = (_cat([o[i, 0], o[i, 1]]) for i in (2 * n, 2 * n + 1))
                        slab, r = divmod(row, 64)
                        if slab < 7:
                            put = ((row, u), (4 * T + row, v))
                        elif slab == 7:
                            put = ((8 * T + r, u), (4 * T + row, sub(v, u)))
                        else:
                            put = ((7 * 64 + r, sub(u, v)), (8 * T + 64 + r, v))
                        for r, w in put:
                            OB[2 * q + n, r:r + 16, :] = _cast(w, bf16)
            return gen(), DH * 64

        return _chain([f(g) for g in range(4) for f in (score, softmax, mix)])

    def project_out(q):
        def gen():
            for g in range(4):
                for n in range(2):
                    both = _dot(_ld(WOP, g, 5), _ld(OB, 2 * q + n, _rows(8, T // 2)))
                    yield DB
                    for i in range(2):
                        acc = both
                        for k in range(4):
                            w = _ld(WOP, g, k if k < 3 else 3 + i)
                            acc = add(acc, _dot(w, _ld(OB, 2 * q + n, _rows(4 * i + k, T // 2))))
                            if k == 3:
                                X1[q][2 * n + i, _rows(g, DB), :] = acc
                            yield DB
        return gen(), 72 * DB

    def slabs(j, among, load):
        if isinstance(j, int):
            return [load(8 if j == t else t) for t in range(8)]
        return [jnp.where(j == t, load(8), load(t)) if t in among else load(t) for t in range(8)]

    def is_chunk(j, n):
        return isinstance(j, int) and j == n

    def w1_transpose(j, s):
        def gen():
            for i in range(4):
                for k in range(4):
                    def load(n):
                        at = _rows(4 * n + k), _rows(i, T)
                        if is_chunk(j, SHARED):
                            return _cast(WS[at], f32)
                        v = _cast(W1R[(s, *at)], f32)
                        return v if n == 8 else sub(v, _cast(WS[at], f32))
                    WT[s, i, k, 0:T, :] = _cat(slabs(j, range(6 - s, 8, 2), load)).T
                    yield 64
        return gen(), 16 * 64

    def w1_last_slab():
        for i in range(4):
            v = W1R[(NC - 1) % 2, 4 * T:D, _rows(i, T)]
            WL[i] = _cat([v, jnp.zeros_like(v)]).T

    def w1_expand(j, s, lo=0, hi=8):
        def gen():
            for t in range(lo, hi):
                def emit(p, v):
                    W1[s][p, _rows(t), :] = v
                yield from _expand(A_TERMS, {(i, k): WT[s, i, k, _rows(t), :] for i in range(4) for k in range(4)}, emit)
                if t % 2 and not is_chunk(j, SHARED):
                    BC[s, t // 2] = to_columns(B1[:, pl.ds(pl.multiple_of(j * FC + t // 2 * T, T), T)])
            traced.append(('w1', s))
        return gen(), (hi - lo) * EXPAND_COST

    def w2_expand(s, lo, hi):
        def gen():
            for t in range(lo, hi):
                blk = {}
                for d in range(4):
                    for k in range(4):
                        blk[d, k] = _cast(W2R[s, _rows(4 * t + d), _rows(k, T)], f32)
                        yield 2

                def emit(p, v):
                    W2[s][p, _rows(t), :] = v
                yield from _expand(A_TERMS, blk, emit)
        return gen(), (hi - lo) * (32 + EXPAND_COST)

    def up(j, s, q):
        extra = 16 if is_chunk(j, NC - 1) else 0

        def gen():
            assert ('w1', s) in traced
            words = HB[q].bitcast(u32)
            for p in range(NP):
                h = _cat(slabs(j, range(4 - s, 7, 2), _once(lambda n: words[p, _rows(n, 8), :])))
                v = _dot(_ld(W1[s], p), pltpu.bitcast(h, bf16))
                if p in ROW_PRODUCTS and not is_chunk(j, SHARED):
                    v = add(v, BC[s, ROW_PRODUCTS.index(p)])
                M1[s][q][product_rows(p), :] = v
                yield T
            for n in range(extra):
                M1[s][q][product_rows(NP + n), :] = _dot(_ld(WL, n // 4), _ld(HB[q], NP + n % 4, slice(0, T // 2)))
                yield T
        return gen(), (NP + extra) * T

    def keep_shared(q):
        def gen():
            for r in range(0, T, 8):
                z = yield from _contract(lambda p: M1[1][q][product_rows(p, r, 8), :])
                for (c, i), v in z.items():
                    Z[q][product_rows(4 * c + i, r, 8), :] = v
                    yield 1
        return gen(), 16 * (2 * NP + 16)

    def activate(j, s, q, lo=0, hi=8):
        rest, at = (M1[s][q], NP) if is_chunk(j, NC - 1) else (Z[q], 0)
        plain = is_chunk(j, NC - 1) and q == NQ - 1

        def gen():
            for t in range(lo, hi):
                halves = []
                for r in (16 * t, 16 * t + 8):
                    pre = yield from _contract(lambda p: M1[s][q][product_rows(p, r, 8), :])
                    for (c, i), u in pre.items():
                        u = add(u, rest[product_rows(at + 4 * c + i, r, 8), :])
                        pre[c, i] = add(mul(u, lax.tanh(mul(u, add(mul(u, u), GK)))), u)
                        yield GELU_COST
                    halves.append(pre)
                blk = {k: _cat([halves[0][k], halves[1][k]]) for k in halves[0]}

                def emit(p, v):
                    GB[s][q][p, _rows(t), :] = v
                if plain:
                    for (c, i), v in blk.items():
                        emit(4 * c + i, _cast(v, bf16))
                else:
                    yield from _expand(B_TERMS, blk, emit)
        return gen(), (hi - lo) * (4 * NP + 32 * GELU_COST + (0 if plain else EXPAND_COST))

    def down(s, q, first=False):
        def gen():
            for p in range(NP):
                v = _dot(_ld(W2[s], p), _ld(GB[s][q], p))
                if not first:
                    v = add(v, ACC[q][p])
                elif p in ROW_PRODUCTS:
                    v = add(v, _cat(MOD[_rows(n, 16, B2), :] for n in range(ROW_PRODUCTS.index(p), D // 16, 4)))
                ACC[q][p] = v
                yield DB
        return gen(), NP * DB

    def finish(q, lo=0, hi=DB // 16):
        def gen():
            for t in range(lo, hi):
                halves = []
                for r in (_rows(2 * t, 8), _rows(2 * t + 1, 8)):
                    halves.append((yield from _contract(lambda p: ACC[q][p, r, :])))
                done = q < NQ - 1 or 64 * t < LAST[2]
                for d in range(4):
                    r = _rows(4 * t + d)
                    gate = MOD[_rows(4 * t + d, 16, GB2), :]
                    for i in range(4):
                        y = add(X1[q][i, r, :], mul(gate, _cat([halves[0][d, i], halves[1][d, i]])))
                        if done:
                            XB[q][i, r, :] = _cast(y, bf16)
                        else:
                            X1[q][i, r, :] = y
                        yield 5
                    if done:
                        collect_across(q, 4 * t + d)
                    yield 12
        return gen(), (hi - lo) * (4 * NP + 16 * 5 + 48)

    def down_last(d):
        q, s, (lo, hi) = NQ - 1, (NC - 1) % 2, LAST[d:d + 2]

        def gen():
            for i in range(4):
                for k in range(4):
                    v = _dot(W2R[s, lo:hi, _rows(k, T)], _ld(GB[s][q], 4 * k + i))
                    acc = v if k == 0 else add(acc, v)
                    yield hi - lo
                y = add(X1[q][i, lo:hi, :], mul(MOD[GB2 + lo:GB2 + hi, :], acc))
                if d < 2:
                    X1[q][i, lo:hi, :] = y
                else:
                    XB[q][i, lo:hi, :] = _cast(y, bf16)
            traced.append(('last', d))
        return gen(), 16 * (hi - lo)

    def send_last(d):
        assert ('last', d) in traced
        for t in range(LAST[d] // 16, LAST[d + 1] // 16):
            collect_across(NQ - 1, t)
        _trace([collect_within(NQ - 1, LAST[d] // 16, LAST[d + 1] // 16)])
        start(f'out3{d}')

    start('c', *x_tiles(0), 'wk0', 'wm0', 'wm1', 'wm2', 'wk1')

    @pl.loop(0, 4)
    def _(n):
        flag[0] = n

    for q in range(NQ):
        HB[q][NP:, 64:T, :] = jnp.zeros((4, 64, T), bf16)

    def block(*lists):
        pl.when(flag[0] >= 0)(lambda: _trace(*lists))

    def ln1(q):
        return [ln1_moments(q), ln1_apply(q)]

    def activate_all(j, s, groups=range(NQ)):
        return [v for q in groups for v in _pieces(activate, j, s, q)]

    shared = [f'ws{n}' for n in range(8)]
    wait('c')
    silu_c()
    wait(*x_tiles(0))
    block([deal_within(0), deal_across(0)])
    wait('wk0')
    block([wqkv_transpose(4, 7), wqkv_expand(1, 0)], [ln1_moments(0)])
    block([_call(ln1_scale, 0)])
    wait('wm0', 'wm1')
    start('wq1', 'wq0')
    block([mod(0, 6), columns(0, 6)])
    wait('wm2')
    start(*x_tiles(1), 'wv')
    block([mod(6, 9), columns(6, 9), ln1_apply(0, True)])
    wait('wk1')
    block([project(0, 1, (0,))], [wqkv_transpose(7, 9), wqkv_expand(1, 1)])
    wait('wq1')
    block([project(0, 1, (1,))], [wqkv_transpose(2, 4), wqkv_expand(0, 1)])
    wait('wq0', *x_tiles(1))
    start(*x_tiles(2))
    block([project(0, 0, (1,))], [wqkv_transpose(0, 2), wqkv_expand(0, 0)], [deal_within(1)])
    wait('wv')
    start(*x_tiles(3))
    block([project(0, 0, (0,))], [wqkv_transpose(9, 14), wqkv_expand(2, 0), deal_across(1)])
    wait(*x_tiles(2))
    start('wo', 'b1', 'b2')
    block([project(0, 2)], [wqkv_expand(2, 1)] + ln1(1), [deal_within(2), deal_across(2)])
    wait(*x_tiles(3), 'wo', 'b1', 'b2')
    block([project(1, 1)], ln1(2), [deal_within(3), first_value(), deal_across(3)], [wo_stage(), _call(biases)])
    block([project(1, 0), project(1, 2), project(2, 1)], [attend(0), wo_transpose()],
          [ln1_moments(3), _call(start, 'wm3', *shared), ln1_apply(3)])
    wait('wm3', *shared)
    chunk(0, 0, 0).start()
    block([project(2, 0), project(2, 2), project_out(0)], [attend(1), w1_transpose(SHARED, 1), columns(9, 24)],
          [mod(9, 24), _idle(900)])
    chunk(0, 0, 0).wait()
    chunk(0, 1, 1).start()
    block([project(3, 0), project(3, 1), project(3, 2), project_out(1)],
          [attend(2), w1_expand(SHARED, 1), ln2_apply(0)], [ln2_moments(0), w1_transpose(0, 0)])
    chunk(1, 0, 0).start()
    chunk(0, 2, 0).start()
    block([project_out(2), up(SHARED, 1, 0), up(0, 0, 0)], [w1_expand(0, 0), attend(3)], [ln2_moments(1)])
    chunk(1, 1, 1).start()
    block([project_out(3)], [ln2_apply(1), ln2_moments(2)], [columns(27, 32)])
    block([up(SHARED, 1, 1), up(0, 0, 1)], [ln2_moments(3), keep_shared(0), ln2_apply(2), ln2_apply(3)])
    chunk(0, 1, 1).wait()
    chunk(1, 0, 0).wait()
    block([up(SHARED, 1, 2), up(SHARED, 1, 3), up(0, 0, 2), up(0, 0, 3)],
          [keep_shared(1)] + _in_turns(activate_all(0, 0, (0, 1)), _pieces(w2_expand, 0, hi=9)), [w1_transpose(1, 1)])
    chunk(0, 3, 1).start()
    chunk(1, 2, 0).start()
    chunk(0, 2, 0).wait()
    block([down(0, 0, True), down(0, 1, True)], [keep_shared(2), w1_expand(1, 1), keep_shared(3)], [w1_transpose(2, 0)])
    chunk(0, 4, 0).start()
    chunk(0, 3, 1).wait()
    chunk(1, 1, 1).wait()
    block([up(1, 1, q) for q in range(NQ)],
          _in_turns(activate_all(0, 0, (2, 3)), _pieces(w1_expand, 2, 0) + _pieces(w2_expand, 1, hi=5)), [w1_transpose(3, 1)])
    chunk(0, 5, 1).start()
    chunk(0, 4, 0).wait()
    start('wm4')
    block([_merge([[up(2, 0, q) for q in range(NQ)], [down(0, 2, True), down(0, 3, True)]], 3)],
          _in_turns(activate_all(1, 1), _pieces(w2_expand, 1, lo=5, hi=9) + _pieces(w1_expand, 3, 1)), [w1_transpose(4, 0)])

    def step(j, s, turn):
        chunk(1, j, s).wait()
        chunk(1, j + 1, 1 - s).start()
        block([_merge([[up(j + 1, 1 - s, q) for q in range(NQ)], [down(1 - s, q) for q in range(NQ)]], RUN)],
              _in_turns(activate_all(j, s), _pieces(w2_expand, s, hi=9) + _pieces(w1_expand, j + 2, s)), [turn])

    @pl.loop(1, 3)
    def _(n):
        j = 2 * n
        chunk(0, j + 3, 1).wait()
        chunk(0, j + 4, 0).start()
        step(j, 0, w1_transpose(j + 3, 1))
        chunk(0, j + 4, 0).wait()
        pl.when(j + 5 < NC)(lambda: chunk(0, j + 5, 1).start())

        @pl.when(j + 4 == NC - 1)
        def _():
            WS[...] = jnp.zeros(WS.shape, bf16)
        step(j + 1, 1, w1_transpose(j + 4, 0))

    step(6, 0, _call(w1_last_slab))
    chunk(1, 7, 1).wait()
    wait('wm4')
    chunk(1, 8, 0).start()
    block([_merge([[up(8, 0, 0), up(8, 0, 1)], [down(0, q) for q in range(NQ)]], 3)],
          _in_turns(activate_all(7, 1)[:-3], _pieces(w2_expand, 1, hi=9)), [mod(24, 27)])
    chunk(1, 8, 0).wait()
    block([_merge([[up(8, 0, 2), up(8, 0, 3)], [down(1, 0)]], 4)],
          _in_turns(activate_all(8, 0, (0, 1)), _pieces(w2_expand, 0, hi=9)))
    block([down(0, 0), down(1, 1)], [activate(8, 0, 2), activate(7, 1, 3, 5, 8)], [columns(24, 27)])
    block([down(0, 1), down(1, 2)], _in_turns(activate_all(8, 0, (3,)), _pieces(finish, 0, hi=9)))
    block([down(0, 2)], [finish(1)], [collect_within(0)])
    start('out0')
    block([down(1, 3)], [finish(2)], [collect_within(1)])
    start('out1')
    block([down_last(0), down_last(1)], [finish(3, 4, 9)], [collect_within(2)])
    start('out2')
    block([down_last(2), down_last(3)],
          [finish(3, 0, 4), collect_within(3, 0, 16), _call(start, 'out31'), _call(send_last, 2), _idle(400)])
    block([_call(send_last, 3)])
    wait(*[k for k in copies if k.startswith('out')])


@jax.jit
def pallas_adaLN_cond__sliding_local_dilated__dense_activation_gelu__prompt_kernel(
    A_x: jax.Array,
    A_wqkv: jax.Array,
    A_wo: jax.Array,
    B_x: jax.Array,
    B_w1: jax.Array,
    B_b1: jax.Array,
    B_w2: jax.Array,
    B_b2: jax.Array,
    c: jax.Array,
    w_mod: jax.Array,
):
    del B_x
    assert A_x.shape == (1, S, D) and B_w1.shape == (D, F)
    vmem = pltpu.VMEM
    scratch = [
        [vmem((4, D, T), bf16)] * NQ,
        vmem((D, 6 * D), bf16),
        vmem((D, 3 * D), bf16),
        vmem((D, D), bf16),
        vmem((2, D, FC), bf16),
        vmem((2, D, FC), bf16),
        vmem((4 * T, FC), bf16),
        vmem((F,), bf16), vmem((D,), bf16), vmem((1, D), bf16),
        vmem((1, F), f32),
        vmem((5 * T, T), f32),
        vmem((D, T), f32),
        vmem((32, 8, T), f32),
        vmem((32 * T, T), f32),
        vmem((6, 18, DB, T), bf16),
        vmem((4, 6, DB, T), bf16),
        vmem((4 * NQ, D // 2, T), u32),
        vmem((2 * NQ, 17, T, T), bf16),
        vmem((4 * NQ, 2, 8, T), f32),
        vmem((NQ, 4, D // 2, T), u32),
        vmem((2 * NQ, 9 * T, T), bf16),
        [vmem((4, D, T), f32)] * NQ,
        [vmem((NP + 4, DB, T), bf16)] * NQ,
        vmem((4, T, T), bf16),
        vmem((2, 4, 4, T + 8, T), f32),
        vmem((2, 4, T, T), f32),
        [vmem((NP, T, T), bf16)] * 2,
        [vmem((NP, DB, T), bf16)] * 2,
        [[vmem(((NP + 16) * (T + 8), T), f32)] * NQ, [vmem((12 * D, T), f32)] * NQ],
        [vmem((16 * (T + 8), T), f32)] * NQ,
        [[vmem((NP, T, T), bf16)] * NQ] * 2,
        [vmem((NP, DB, T), f32)] * NQ,
        pltpu.SMEM((1,), jnp.int32),
        pltpu.SemaphoreType.DMA((44,)),
        pltpu.SemaphoreType.DMA((4,)),
    ]
    out = pl.pallas_call(
        _kernel,
        out_shape=jax.ShapeDtypeStruct((D, S), A_x.dtype),
        in_specs=[pl.BlockSpec(memory_space=pl.ANY)] * 9,
        out_specs=pl.BlockSpec(memory_space=pl.ANY),
        scratch_shapes=scratch,
        compiler_params=pltpu.CompilerParams(
            vmem_limit_bytes=124 * 2**20,
            flags={'XLA_TPU_EVENLY_DISTRIBUTE_CRITICAL_NODES': True}),
        name='adaln_block',
    )(A_x.reshape(S, D).T, A_wqkv, A_wo, B_w1, B_b1, B_w2.T, B_b2, c, w_mod)
    return out.T.reshape(1, S, D)
```
